```python
import os as _os
_os.environ.setdefault("JAX_PLATFORMS", "cpu")
import jax
import jax.numpy as jnp

def _softmax(x, axis=-1):
    return jax.nn.softmax(x, axis=axis)
def _gelu(x):
    return jax.nn.gelu(x, approximate=True)
def _silu(x):
    return jax.nn.silu(x)
def _sigmoid(x):
    return jax.nn.sigmoid(x)
def _layernorm(x, axis=-1, eps=1e-5):
    m = jnp.mean(x, axis=axis, keepdims=True)
    v = jnp.var(x, axis=axis, keepdims=True)
    return (x - m) / jnp.sqrt(v + eps)
def _scatter_add(tgt, idx, src, axis=0):
    return tgt.at[idx].add(src)
def _segment_sum(src, seg, n):
    return jax.ops.segment_sum(src, seg, n)
class _Rng:
    def __init__(self, key):
        self._k = key
    def _next(self):
        self._k, sub = jax.random.split(self._k)
        return sub
    def normal(self, shape):
        return jax.random.normal(self._next(), shape, dtype=jnp.bfloat16)
    def randint(self, lo, hi, shape):
        return jax.random.randint(self._next(), shape, lo, hi, dtype=jnp.int32)
    def uniform(self, shape, lo=0.0, hi=1.0):
        return jax.random.uniform(self._next(), shape, jnp.bfloat16, lo, hi)
    def permutation(self, n):
        return jax.random.permutation(self._next(), n)


kernel_name = 'interleave_layers__grouped_kv_mqa__sliding_block__prompt'

def setup_inputs():
    _rng = _Rng(jax.random.key(int.from_bytes(__import__("os").urandom(4), "little")))
    _w = (lambda a: (lambda t: t.astype(jnp.bfloat16) if jnp.issubdtype(t.dtype, jnp.floating) else t)(jnp.asarray(a)))
    def _A_setup():
        B, S, D, H = 1, 2048, 448, 16
        Dh = D // H
        return {
            "x": _w((lambda *s: _rng.normal(s) * 0.05)(B, S, D)),
            "wq": _w((lambda *s: _rng.normal(s) * 0.05)(D, H * Dh)),
            "wk": _w((lambda *s: _rng.normal(s) * 0.05)(D, Dh)),
            "wv": _w((lambda *s: _rng.normal(s) * 0.05)(D, Dh)),
            "wo": _w((lambda *s: _rng.normal(s) * 0.05)(H * Dh, D)),
        }
    _A_in = _A_setup()

    def _B_setup():
        B, S, D = 1, 2048, 448
        return {
            "x": _w((lambda *s: _rng.normal(s) * 0.05)(B, S, D)),
            "wqkv": _w((lambda *s: _rng.normal(s) * 0.05)(D, 3 * D)),
            "wo": _w((lambda *s: _rng.normal(s) * 0.05)(D, D)),
        }
    _B_in = _B_setup()

    return {
        "A_x": _A_in["x"],
        "A_wq": _A_in["wq"],
        "A_wk": _A_in["wk"],
        "A_wv": _A_in["wv"],
        "A_wo": _A_in["wo"],
        "B_x": _B_in["x"],
        "B_wqkv": _B_in["wqkv"],
        "B_wo": _B_in["wo"],
    }

def reference(A_x, A_wq, A_wk, A_wv, A_wo, B_x, B_wqkv, B_wo):
    def _A_ref(x, wq, wk, wv, wo):
        B, S, D = x.shape
        H = 16
        Dh = D // H
        q = (lambda x, *d: x.transpose(*d))((x @ wq).reshape(B, S, H, Dh), 0, 2, 1, 3)
        k = x @ wk
        v = x @ wv
        scores = jnp.einsum("bhqd,bkd->bhqk", q, k) * (Dh ** -0.5)
        p = _softmax(scores, axis=-1)
        o = jnp.einsum("bhqk,bkd->bhqd", p, v)
        return (lambda x, *d: x.transpose(*d))(o, 0, 2, 1, 3).reshape(B, S, H * Dh) @ wo

    def _B_ref(x, wqkv, wo):
        B, S, D = x.shape
        H = 16; Dh = D // H; W = 256
        qkv = (lambda x, *d: x.transpose(*d))((x @ wqkv).reshape(B, S, 3, H, Dh), 2, 0, 3, 1, 4)
        q, k, v = qkv[0], qkv[1], qkv[2]
        scores = jnp.einsum("bhqd,bhkd->bhqk", q, k) * (Dh ** -0.5)
        idx = jnp.arange(S)
        mask = (idx[:, None] - idx[None, :] >= 0) & (idx[:, None] - idx[None, :] < W)
        scores = jnp.where(mask[None, None], scores, -1e9)
        p = _softmax(scores, axis=-1)
        o = jnp.einsum("bhqk,bhkd->bhqd", p, v)
        return (lambda x, *d: x.transpose(*d))(o, 0, 2, 1, 3).reshape(B, S, D) @ wo

    x = A_x
    x = x + _A_ref(_layernorm(x, axis=-1), A_wq, A_wk, A_wv, A_wo)
    x = x + _B_ref(_layernorm(x, axis=-1), B_wqkv, B_wo)
    x = x + _A_ref(_layernorm(x, axis=-1), A_wq, A_wk, A_wv, A_wo)
    x = x + _B_ref(_layernorm(x, axis=-1), B_wqkv, B_wo)
    return x
```

```python
import functools
import math

import jax
import jax.numpy as jnp
from jax import lax
import jax.experimental.pallas as pl
import jax.experimental.pallas.tpu as pltpu

S, D, H, DH, WIN = 2048, 448, 16, 28, 256
T = 128
NT = S // T
HG = 4
NG = H // HG
GR = HG * DH
QSCALE = (DH ** -0.5) * math.log2(math.e)
NEG = -1e30
F32, BF16 = jnp.float32, jnp.bfloat16


def _dot(a, b):
    return jnp.dot(a, b, preferred_element_type=F32)


def _layernorm_t(x):
    m = jnp.sum(x, axis=0, keepdims=True) * (1.0 / D)
    d = x - m
    v = jnp.sum(d * d, axis=0, keepdims=True) * (1.0 / D)
    return d * lax.rsqrt(v + 1e-5)


def kernel(x_ref, wq_ref, wkT_ref, wvT_ref, woA_ref, wqkv_ref, woB_ref, out_ref,
           xres, wA, woAT, wB, woBT, s_buf, m_buf, o_buf, qA, kA, vA, qB, kB, vB):
    wA[0:D, :] = wq_ref[...].T
    wA[D:D + 64, :] = jnp.concatenate(
        [wkT_ref[...].astype(F32), wvT_ref[...].astype(F32), jnp.zeros((8, D), F32)], axis=0).astype(BF16)
    woAT[...] = woA_ref[...].T
    wB[...] = wqkv_ref[...].T
    woBT[...] = woB_ref[...].T
    kB[:, 0:WIN, :] = jnp.zeros((NG, WIN, 128), BF16)
    vB[:, 0:WIN] = jnp.zeros((H * 32, WIN), BF16)

    def tcols(t):
        return pl.ds(pl.multiple_of(t * T, T), T)

    def proj_a(t, xn):
        y = _dot(wA[...], xn)
        q = y[0:D] * QSCALE
        z4 = jnp.zeros((4, T), F32)
        for h in range(H):
            qh = jnp.concatenate([q[h * DH:(h + 1) * DH], z4], axis=0)
            qA[:, pl.ds(pl.multiple_of(t * (H * T) + h * T, T), T)] = qh.astype(BF16)
        kT = jnp.concatenate([y[D:D + DH], jnp.zeros((128 - DH, T), F32)], axis=0)
        kA[tcols(t), :] = kT.T[:, 0:32].astype(BF16)
        vA[:, tcols(t)] = jnp.concatenate([y[D + DH:D + 2 * DH], jnp.ones((4, T), F32)], axis=0).astype(BF16)

    def proj_b(t, xn):
        y = _dot(wB[...], xn)
        q = y[0:D] * QSCALE
        for g in range(NG):
            for j in range(HG):
                h = g * HG + j
                parts = []
                if j > 0:
                    parts.append(jnp.zeros((j * DH, T), F32))
                parts.append(q[h * DH:(h + 1) * DH])
                parts.append(jnp.zeros((128 - (j + 1) * DH, T), F32))
                qB[g, :, pl.ds(pl.multiple_of(t * (HG * T) + j * T, T), T)] = jnp.concatenate(parts, axis=0).astype(BF16)
            kT = y[D + g * GR:D + g * GR + 128]
            kB[g, pl.ds(pl.multiple_of(t * T + WIN, T), T), :] = kT.T.astype(BF16)
        o4 = jnp.ones((4, T), F32)
        for h in range(H):
            vh = jnp.concatenate([y[2 * D + h * DH:2 * D + (h + 1) * DH], o4], axis=0)
            vB[h * 32:(h + 1) * 32, pl.ds(pl.multiple_of(t * T + WIN, T), T)] = vh.astype(BF16)

    def post(t, woT):
        y = _dot(woT[...], o_buf[...])
        x = xres[:, tcols(t)] + y
        xres[:, tcols(t)] = x
        return x

    def finish_group(g, acc):
        on = acc[0:DH] * pl.reciprocal(acc[DH:DH + 1])
        o_buf[g * GR:(g + 1) * GR, :] = jnp.concatenate(
            [on[:, j * T:(j + 1) * T] for j in range(HG)], axis=0).astype(BF16)

    def attn_a(t, do_qk, do_pv):
        for g in range(NG):
            lc = pl.ds(g * HG * T, HG * T)
            if do_qk:
                q = qA[:, pl.ds(pl.multiple_of(t * (H * T) + g * HG * T, HG * T), HG * T)]
            if do_pv:
                m_prev = m_buf[0:1, lc]
            m_new = acc = None
            for c in range(NT):
                rows = pl.ds(c * T, T)
                if do_pv:
                    p = jnp.exp2(s_buf[rows, lc] - m_prev).astype(BF16)
                if do_qk:
                    s = _dot(kA[rows, :], q)
                    s_buf[rows, lc] = s
                    mc = jnp.max(s.reshape(T // 8, 8, HG * T), axis=0)
                    m_new = mc if m_new is None else jnp.maximum(m_new, mc)
                if do_pv:
                    o = _dot(vA[:, rows], p)
                    acc = o if acc is None else acc + o
            if do_pv:
                finish_group(g, acc)
            if do_qk:
                m_buf[0:1, lc] = jnp.max(m_new, axis=0, keepdims=True)

    def attn_b(t, do_qk, do_pv):
        a = lax.broadcasted_iota(jnp.int32, (T, HG * T), 0)
        b = lax.broadcasted_iota(jnp.int32, (T, HG * T), 1) % T
        for g in range(NG):
            lc = pl.ds(g * HG * T, HG * T)
            if do_qk:
                q = qB[g, :, pl.ds(pl.multiple_of(t * (HG * T), HG * T), HG * T)]
            if do_pv:
                m_prev = m_buf[0:1, lc]
            m_new = None
            acc = [None] * HG
            for c in range(3):
                rows = pl.ds(c * T, T)
                if do_pv:
                    p = jnp.exp2(s_buf[rows, lc] - m_prev).astype(BF16)
                if do_qk:
                    s = _dot(kB[g, pl.ds(pl.multiple_of((t + c) * T, T), T), :], q)
                    if c == 0:
                        s = jnp.where(a > b + jnp.where(t >= 2, 0, T), s, NEG)
                    elif c == 1:
                        s = jnp.where(a >= jnp.where(t >= 1, 0, T), s, NEG)
                    else:
                        s = jnp.where(a <= b, s, NEG)
                    s_buf[rows, lc] = s
                    mc = jnp.max(s.reshape(T // 8, 8, HG * T), axis=0)
                    m_new = mc if m_new is None else jnp.maximum(m_new, mc)
                if do_pv:
                    for j in range(HG):
                        h = g * HG + j
                        o = _dot(vB[h * 32:(h + 1) * 32, pl.ds(pl.multiple_of((t - 1 + c) * T, T), T)],
                                 p[:, j * T:(j + 1) * T])
                        acc[j] = o if acc[j] is None else acc[j] + o
            if do_pv:
                finish_group(g, jnp.concatenate(acc, axis=1))
            if do_qk:
                m_buf[0:1, lc] = jnp.max(m_new, axis=0, keepdims=True)

    def first(t, c):
        x = x_ref[:, tcols(t)].astype(F32)
        xres[:, tcols(t)] = x
        proj_a(t, _layernorm_t(x).astype(BF16))
        return c
    lax.fori_loop(0, NT, first, 0)

    def pair(r, c):
        attn_a(0, True, False)

        def a_body(t, c):
            attn_a(t, True, True)
            x = post(t - 1, woAT)
            proj_b(t - 1, _layernorm_t(x).astype(BF16))
            return c
        lax.fori_loop(1, NT, a_body, 0)
        attn_a(NT, False, True)
        x = post(NT - 1, woAT)
        proj_b(NT - 1, _layernorm_t(x).astype(BF16))

        attn_b(0, True, False)

        def b_tail(t):
            x = post(t, woBT)

            @pl.when(r == 0)
            def _():
                proj_a(t, _layernorm_t(x).astype(BF16))

            @pl.when(r == 1)
            def _():
                out_ref[:, tcols(t)] = x.astype(BF16)

        def b_body(t, c):
            attn_b(t, True, True)
            b_tail(t - 1)
            return c
        lax.fori_loop(1, NT, b_body, 0)
        attn_b(NT, False, True)
        b_tail(NT - 1)
        return c
    lax.fori_loop(0, 2, pair, 0)


@jax.jit
def pallas_interleave_layers__grouped_kv_mqa__sliding_block__prompt_kernel(A_x, A_wq, A_wk, A_wv, A_wo, B_x, B_wqkv, B_wo):
    del B_x
    xT = jnp.swapaxes(A_x[0], 0, 1)
    outT = pl.pallas_call(
        kernel,
        out_shape=jax.ShapeDtypeStruct((D, S), BF16),
        scratch_shapes=[
            pltpu.VMEM((D, S), F32),
            pltpu.VMEM((D + 64, D), BF16),
            pltpu.VMEM((D, D), BF16),
            pltpu.VMEM((3 * D, D), BF16),
            pltpu.VMEM((D, D), BF16),
            pltpu.VMEM((S, H * T), F32),
            pltpu.VMEM((8, H * T), F32),
            pltpu.VMEM((D, T), BF16),
            pltpu.VMEM((32, H * S), BF16),
            pltpu.VMEM((S, 32), BF16),
            pltpu.VMEM((32, S), BF16),
            pltpu.VMEM((NG, 128, HG * S), BF16),
            pltpu.VMEM((NG, S + WIN, 128), BF16),
            pltpu.VMEM((H * 32, S + WIN), BF16),
        ],
        compiler_params=pltpu.CompilerParams(vmem_limit_bytes=100 * 1024 * 1024),
        name="fused_layers",
    )(xT, A_wq, A_wk.T, A_wv.T, A_wo, B_wqkv, B_wo)
    return jnp.swapaxes(outT, 0, 1)[None]
```

```python
import math

import jax
import jax.numpy as jnp
from jax import lax
import jax.experimental.pallas as pl
import jax.experimental.pallas.tpu as pltpu

S, D, H, DH, WIN = 2048, 448, 16, 28, 256
T = 128
NT = S // T
HG = 4
NG = H // HG
GR = HG * DH
GW = HG * T
XC = 4
NV = 192
NV0 = min(NV, 128)
BAND = WIN + 32
QSCALE = (DH ** -0.5) * math.log2(math.e)
NEG = -1e30
L_MIN, L_MAX = 2.0 ** -60, 2.0 ** 100
F32, BF16, I32 = jnp.float32, jnp.bfloat16, jnp.int32
D_ORDER = sorted(range(DH), key=lambda d: (d % 8, d // 8))


def _dot(a, b):
    return jnp.dot(a, b, preferred_element_type=F32)


def _pack(x):
    r, c = x.shape
    if c > 128:
        return pltpu.bitcast(x.astype(BF16), I32)
    w = pltpu.bitcast(jnp.concatenate([x[i:i + 16] for i in range(0, r, 16)], axis=1).astype(BF16), I32)
    return jnp.concatenate([w[:, i:i + c] for i in range(0, w.shape[1], c)], axis=0)


def _unpack(x):
    return pltpu.bitcast(x, BF16)


def _tree(op, xs):
    xs = list(xs)
    while len(xs) > 1:
        xs = [op(xs[i], xs[i + 1]) if i + 1 < len(xs) else xs[i] for i in range(0, len(xs), 2)]
    return xs[0]


def _colsum(x):
    return jnp.sum(_tree(jnp.add, [x[i:i + 8] for i in range(0, x.shape[0], 8)]), axis=0, keepdims=True)


def _ds(start, size, mult=T):
    if isinstance(start, int):
        return pl.ds(start, size)
    return pl.ds(pl.multiple_of(start, mult), size)


def _weave(main, extras):
    for i, item in enumerate(main):
        for e in extras.get(i, ()):
            e()
        item()
    for i in sorted(extras):
        if i >= len(main):
            for e in extras[i]:
                e()


def _spread(items, start, stride):
    out = {}
    for i, it in enumerate(items):
        out.setdefault(start + int(i * stride), []).append(it)
    return out


import contextlib
def scope(name):
    return contextlib.nullcontext()


def _merge(*ds):
    out = {}
    for d in ds:
        for k, v in d.items():
            out.setdefault(k, []).extend(v)
    return out


def kernel(x_hbm, wq_hbm, wk_hbm, wv_hbm, woA_hbm, wqkv_hbm, woB_hbm, out_hbm,
           x_in, wq_in, wk_in, wv_in, woA_in, wqkv_in, woB_in, out_st, in_sem, out_sem,
           xres, xn_buf, wA, woAT, wB, woBT, pA, pB, o_buf, chk, qmask,
           qA, qF, kA, vA, qB, kB, kY, vB, sX, *ops):
    XW = S // XC
    x_cp = [pltpu.make_async_copy(x_hbm.at[:, pl.ds(i * XW, XW)], x_in.at[:, pl.ds(i * XW, XW)], in_sem.at[i])
            for i in range(XC)]
    w_cp = [pltpu.make_async_copy(src, dst, in_sem.at[XC + i]) for i, (src, dst) in enumerate(
        [(wk_hbm, wk_in), (wv_hbm, wv_in), (wq_hbm, wq_in), (woA_hbm, woA_in), (wqkv_hbm, wqkv_in), (woB_hbm, woB_in)])]
    for c in (w_cp[0], w_cp[1], x_cp[0], w_cp[2], *x_cp[1:], *w_cp[3:]):
        c.start()

    def out_copy(t):
        return pltpu.make_async_copy(out_st.at[:, _ds(t * T, T)], out_hbm.at[:, _ds(t * T, T)], out_sem.at[0])

    def lane_bit(width, bit):
        return ((lax.broadcasted_iota(I32, (8, 128), 1) // width) & bit) != 0

    def pick(mask, a, b):
        r = a.shape[0]
        return jnp.where(mask[None], a.reshape(r // 8, 8, 128), b.reshape(r // 8, 8, 128)).reshape(r, 128)

    def wdot(w_ref, r0, n):
        return _dot(_unpack(w_ref[pl.ds(r0 // 2, n // 2), :]), _unpack(xn_buf[...]))

    def ln_items(t):
        st = {}

        def mean():
            st["m"] = _colsum(xres[:, _ds(t * T, T)]) * (1.0 / D)

        def var():
            d = xres[:, _ds(t * T, T)] - st["m"]
            st["r"] = lax.rsqrt(_colsum(d * d) * (1.0 / D) + 1e-5)

        def norm():
            xn_buf[...] = _pack((xres[:, _ds(t * T, T)] - st["m"]) * st["r"])
        return [mean, var, norm]

    def load_x(t):
        def f():
            xres[:, _ds(t * T, T)] = x_in[:, _ds(t * T, T)].astype(F32)
        return f

    def proj_a_items(t):
        def kv():
            y = wdot(wA, D, 64)
            kT = jnp.concatenate([y[0:DH], jnp.zeros((128 - DH, T), F32)], axis=0)
            kA[_ds(t * (T // 2), T // 2, T // 2), :] = _pack(kT.T)[:, 0:32]
            vA[:, _ds(t * T, T)] = _pack(jnp.concatenate([y[DH:2 * DH], jnp.ones((4, T), F32)], axis=0))

        def q(g):
            def f():
                y = wdot(wA, g * GR, GR) * QSCALE
                z4 = jnp.zeros((4, T), F32)
                qg = jnp.concatenate(
                    [jnp.concatenate([y[j * DH:(j + 1) * DH], z4], axis=0) for j in range(HG)], axis=1)
                cols = _ds(t * (H * T) + g * GW, GW)
                qA[:, cols] = _pack(qg)
                if NV: qF[:, cols] = qg
            return f
        return [kv] + [q(g) for g in range(NG)]

    def key_bcast_items():
        def one(kb):
            def f():
                k = _unpack(kA[pl.ds(kb * 8, 8), :]).astype(F32)
                for d in range(DH):
                    b = jnp.broadcast_to(k[:, d:d + 1], (16, 128))
                    c0 = H * T + (kb * 8 + d % 8) * 256
                    ops[d // 8][:, pl.ds(c0, 256)] = jnp.concatenate([b[0:8], b[8:16]], axis=1)
            return f
        return [one(kb) for kb in range(NV // 16)]

    def proj_b_items(t):
        def k(g):
            def f():
                y = wdot(wB, D + g * GR, GR)
                kT = jnp.concatenate([y, jnp.zeros((128 - GR, T), F32)], axis=0)
                cur = _pack(kT.T)
                kB[g, _ds(t * (T // 2) + WIN // 2, T // 2, T // 2), :] = cur
                w = jnp.concatenate([kB[g, _ds(t * (T // 2) + (WIN - 96) // 2, 48, 16), :], cur], axis=0)
                b0, b1 = lane_bit(DH, 1), lane_bit(DH, 2)
                z = [pick(b0, w[16:112], w[0:96]), pick(b0, w[0:96], w[16:112])]
                rows = _ds(t * (T // 2) + 80, T // 2, 16)
                for a in range(2):
                    kY[g, a, rows, :] = pick(b1, z[a][32:96], z[a][0:64])
                    kY[g, a + 2, rows, :] = pick(b1, z[a][0:64], z[a][32:96])
            return f

        def q(g):
            def f():
                qB[pl.ds(g * GR // 2, GR // 2), _ds(t * T, T)] = _pack(wdot(wB, g * GR, GR) * QSCALE)
            return f

        def v(g):
            def f():
                y = wdot(wB, 2 * D + g * GR, GR)
                o4 = jnp.ones((4, T), F32)
                parts = []
                for j in range(HG):
                    parts += [y[j * DH:(j + 1) * DH], o4]
                vB[pl.ds(g * 64, 64), _ds(t * T + WIN, T)] = _pack(jnp.concatenate(parts, axis=0))
            return f
        return [k(g) for g in range(NG)] + [q(g) for g in range(NG)] + [v(g) for g in range(NG)]

    def out_items(t, woT, last=False):
        def part(g):
            def f():
                rows = pl.ds(g * GR, GR)
                y = _dot(_unpack(woT[pl.ds(g * GR // 2, GR // 2), :]), _unpack(o_buf[...]))
                x = xres[rows, _ds(t * T, T)] + y
                if last:
                    out_st[rows, _ds(t * T, T)] = x.astype(BF16)
                else:
                    xres[rows, _ds(t * T, T)] = x
            return f
        items = [part(g) for g in range(NG)]
        if last:
            items.append(lambda: out_copy(t).start())
        return items

    def store_o(g, acc):
        on = acc[0:DH] * pl.reciprocal(acc[DH:DH + 1])
        o_buf[_ds(g * (GR // 2), GR // 2, 8), :] = _pack(
            jnp.concatenate([on[:, j * T:(j + 1) * T] for j in range(HG)], axis=0))

    def finish_group(g, acc):
        store_o(g, acc)
        den = [acc[24:32, j * T:(j + 1) * T] for j in range(HG)]
        chk[0:8] = chk[0:8] + _tree(jnp.add, [acc[i:i + 8, j * T:(j + 1) * T] for i in range(0, 32, 8) for j in range(HG)])
        chk[8:16] = jnp.minimum(chk[8:16], _tree(jnp.minimum, den))
        chk[16:24] = jnp.maximum(chk[16:24], _tree(jnp.maximum, den))

    def attn_a_items(t, do_qk, do_pv, zero, tail=0, nv=NV):
        st, cur = {}, {}
        steps = [(g, c) for g in range(NG) for c in range(NT)]

        def pv(g, c):
            p = _unpack(pA[pl.ds(c * (T // 2), T // 2), pl.ds(g * GW, GW)])
            o = _dot(_unpack(vA[:, pl.ds(c * T, T)]), p)
            st["o"] = o
            st["acc"] = o if c == 0 else st["acc"] + o
            if c == NT - 1:
                finish_group(g, st["acc"])

        def qk(g, c):
            if c == 0:
                st["q"] = _unpack(qA[:, _ds(t * (H * T) + g * GW, GW)])
            lo, hi = (nv + (S - nv) * i // NT // 16 * 16 for i in (c, c + 1))
            rows = pl.ds(lo // 2, (hi - lo) // 2)
            st["s"] = s = _dot(_unpack(kA[rows, :]), st["q"])
            pA[rows, pl.ds(g * GW, GW)] = _pack(jnp.exp2(s))

        def vpu_block(g, kb):
            a = {}

            def one(n, d):
                def f():
                    buf = ops[d // 8]
                    if "v" in cur:
                        buf[:, _ds(zero + (OPW - 128), 128)] = cur["v"]
                    kk = buf[:, pl.ds(H * T + (kb * 8 + d % 8) * 256, 256)]
                    kk = jnp.concatenate([kk[:, 0:128], kk[:, 128:256]], axis=0)
                    term = jnp.concatenate([kk] * HG, axis=1) * buf[d % 8:d % 8 + 1, pl.ds(g * GW, GW)]
                    a["s"] = term if n == 0 else a["s"] + term
                    if n == DH - 1:
                        pA[pl.ds(kb * 8, 8), pl.ds(g * GW, GW)] = _pack(jnp.exp2(a["s"]))
                return f
            return [one(n, d) for n, d in enumerate(D_ORDER)]

        side = []
        if do_qk:
            side = [(g, f) for g in range(NG) for kb in range(nv // 16) for f in vpu_block(g, kb)]
        ahead = -(-nv // T) if do_qk and do_pv else 0
        per_step = (16 if do_qk else 0) + (4 if do_pv else 0)
        total = len(steps) * per_step - tail
        prog = {"slot": 0, "done": 0, "pv": 0}

        def tick(v):
            cur["v"] = v
            prog["slot"] += 1
            want = min(len(side), len(side) * prog["slot"] // total)
            while prog["done"] < want and (not do_pv or prog["pv"] >= min(len(steps), side[prog["done"]][0] * NT + ahead)):
                side[prog["done"]][1]()
                prog["done"] += 1

        def step(n):
            def f():
                if NV and do_qk and n == 0:
                    for b in range(4):
                        ops[b][:, 0:H * T] = qF[pl.ds(b * 8, 8), _ds(t * (H * T), H * T)]
                pvs = []
                if do_pv:
                    pvs = list(range(ahead + 1)) if n == 0 else [n + ahead] if n + ahead < len(steps) else []
                for i in pvs:
                    pv(*steps[i])
                    prog["pv"] = i + 1
                    for a in range(0, 32, 8):
                        tick(st["o"][a:a + 8, 0:128])
                if do_qk:
                    qk(*steps[n])
                    nr = st["s"].shape[0]
                    for a in range(16):
                        r = a * nr // 128 * 8
                        tick(st["s"][r:r + 8, 0:128])
                if n == len(steps) - 1:
                    for _, rest in side[prog["done"]:]:
                        rest()
            return f
        return [step(n) for n in range(len(steps))]

    def attn_b_items(t, qk_b0, pv_c0):
        def pv(g):
            odd, high = lane_bit(32, 1), lane_bit(32, 2)
            A = [pB[g, u] for u in range(4)]
            zb = jnp.zeros((16, 128), I32)
            B = [pick(odd, jnp.concatenate([zb, A[a ^ 1]], axis=0), jnp.concatenate([A[a], zb], axis=0))
                 for a in range(4)]
            r0 = pv_c0 * 64
            outs = []
            for h in range(HG):
                y = pick(high, jnp.concatenate([zb, zb, B[h ^ 2]], axis=0)[r0:],
                         jnp.concatenate([B[h], zb, zb], axis=0)[r0:])
                v = vB[pl.ds((g * HG + h) * 16, 16), _ds((t - 1 + pv_c0) * T, (3 - pv_c0) * T)]
                outs.append(_dot(_unpack(v), _unpack(y)))
            finish_group(g, jnp.concatenate(outs, axis=1))

        def qk(g):
            qg = qB[pl.ds(g * GR // 2, GR // 2), _ds(t * T, T)]
            r0 = qk_b0 * 16
            n = BAND // 2 - r0
            for u in range(4):
                s = _dot(_unpack(kY[g, u, _ds(t * (T // 2) + r0, n, 16), 0:GR]), _unpack(qg & qmask[u]))
                p = _pack(jnp.exp2(s))
                parts = [p[16:n - 16] if qk_b0 == 0 else p[0:n - 16], p[n - 16:n] & qmask[5, 0:16]]
                if qk_b0 == 0:
                    parts = [p[0:16] & qmask[4, 0:16]] + parts
                pB[g, u, pl.ds(r0, n), :] = jnp.concatenate(parts, axis=0)

        def step(g):
            def f():
                if pv_c0 is not None:
                    pv(g)
                if qk_b0 is not None:
                    qk(g)
            return f
        return [step(g) for g in range(NG)]

    def post_a(t, p_out=0, p_ln=1, p_proj=6, stride=4):
        return _merge({p_out: out_items(t, woAT)}, _spread(ln_items(t), p_ln, 1),
                      _spread(proj_b_items(t), p_proj, stride))

    def post_b(t, last, p_out=0, p_ln=1, p_proj=2, stride=0.5):
        if last:
            return {p_out: out_items(t, woBT, True)}
        pa = proj_a_items(t)
        dbg = ""
        if dbg == "nokv": pa = pa[1:]
        if dbg == "noq": pa = pa[:1]
        return _merge({p_out: out_items(t, woBT)}, _spread(ln_items(t), p_ln, 0),
                      _spread(pa, p_proj, stride))

    row = lax.broadcasted_iota(I32, (GR // 2, 128), 0)
    lane = lax.broadcasted_iota(I32, (GR // 2, 128), 1)
    for u in range(4):
        qmask[u] = jnp.where(((row // (DH // 2)) ^ (lane // 32)) == u, -1, 0)
    lo_w, hi_w = 0xFFFF, -0x10000
    qmask[4] = jnp.where(2 * row > lane % 32, lo_w, 0) | jnp.where(2 * row + 1 > lane % 32, hi_w, 0)
    qmask[5] = jnp.where(2 * row <= lane % 32, lo_w, 0) | jnp.where(2 * row + 1 <= lane % 32, hi_w, 0)
    chk[0:8] = jnp.zeros((8, 128), F32)
    chk[8:24] = jnp.ones((16, 128), F32)
    kB[:, 0:WIN // 2, :] = jnp.zeros((NG, WIN // 2, 128), I32)
    kY[:, :, 0:80, :] = jnp.zeros((NG, 4, 80, 128), I32)
    pB[:, :, 0:80, :] = jnp.zeros((NG, 4, 80, 128), I32)
    vB[:, 0:WIN] = jnp.zeros((H * 16, WIN), I32)

    w_cp[0].wait()
    w_cp[1].wait()
    wA[D // 2:D // 2 + 32, :] = _pack(jnp.concatenate(
        [wk_in[...].astype(F32), wv_in[...].astype(F32), jnp.zeros((8, D), F32)], axis=0))
    x_cp[0].wait()
    load_x(0)()
    for it in ln_items(0):
        it()
    w_cp[2].wait()
    wA[0:D // 2, :] = _pack(wq_in[...].T)
    kbi = key_bcast_items()
    for t in range(NT):
      with scope("proA"):
        items = proj_a_items(t)
        extra = {}
        if t + 1 < NT:
            if (t + 1) % (NT // XC) == 0:
                x_cp[(t + 1) // (NT // XC)].wait()
            ln = ln_items(t + 1)
            extra = {0: [load_x(t + 1), ln[0]], 1: [ln[1]], len(items): [ln[2]]}
        if t >= 2:
            extra = _merge(extra, {2: kbi[len(kbi) * (t - 2) // (NT - 2):len(kbi) * (t - 1) // (NT - 2)]})
        _weave(items, extra)

    def prep(cp, src, dst):
        def f():
            cp.wait()
            dst[...] = _pack(src[...].T)
        return f

    opaque0 = jnp.max(chk[0:8]).astype(I32) * 128
    for r in range(2):
        last = r == 1
        if r == 0:
          with scope("qk0"):
            _weave(attn_a_items(0, True, False, opaque0, nv=NV0),
                   {8: [prep(w_cp[3], woA_in, woAT)], 16: [prep(w_cp[4], wqkv_in, wB)],
                    48: [prep(w_cp[5], woB_in, woBT)]})
        with scope(f"a1_{r}"):
            _weave(attn_a_items(1, True, True, opaque0), {})

        def a_body(i, c):
            _weave(attn_a_items(i, True, True, (i >> 20) * 128), post_a(i - 2))
            return c
        with scope(f"aloop_{r}"):
            lax.fori_loop(2, NT, a_body, 0)

        with scope(f"ab_{r}"):
            _weave(attn_a_items(None, False, True, opaque0),
               _merge(post_a(NT - 2, stride=3), _spread(attn_b_items(0, 5, None), 44, 4)))
            _weave(attn_b_items(1, 1, 2), post_a(NT - 1, p_ln=1, p_proj=4, stride=0))
            _weave(attn_b_items(2, 0, 1), post_b(0, last))

        def b_body(i, c):
            _weave(attn_b_items(i, 0, 0), post_b(i - 2, last))
            return c
        with scope(f"bloop_{r}"):
            lax.fori_loop(3, NT, b_body, 0)

        with scope(f"ba_{r}"):
            _weave(attn_b_items(NT, None, 0), _merge(post_b(NT - 2, last), {} if last else _spread(key_bcast_items(), 0, 4 / max(1, NV // 16))))
            if last:
                _weave([], post_b(NT - 1, last))
            else:
                _weave(attn_a_items(0, True, False, opaque0, nv=NV0), post_b(NT - 1, last, p_proj=6, stride=1))
    for t in range(NT):
        out_copy(t).wait()

    sub = lax.broadcasted_iota(I32, (8, 128), 0)
    ok = (jnp.abs(chk[0:8]) < float("inf")) & (((chk[8:16] >= L_MIN) & (chk[16:24] <= L_MAX)) | (sub < 4))

    @pl.when(jnp.min(jnp.where(ok, 1.0, 0.0)) < 0.5)
    def _():
        def run(items):
            for it in items:
                it()

        def first(t, c):
            run([load_x(t)] + ln_items(t) + proj_a_items(t))
            return c
        lax.fori_loop(0, NT, first, 0)

        def a_tile(t, c):
            def group(g, c):
                q = _unpack(qA[:, _ds(t * (H * T) + g * GW, GW)])

                def scores(k, m):
                    s = _dot(_unpack(kA[_ds(k * 64, 64, 64), :]), q)
                    sX[_ds(k * T, T), :] = s
                    return jnp.maximum(m, jnp.max(s, axis=0, keepdims=True))
                m = lax.fori_loop(0, NT, scores, jnp.full((1, GW), -jnp.inf, F32))

                def pv(k, acc):
                    p = jnp.exp2(sX[_ds(k * T, T), :] - m).astype(BF16)
                    return acc + _dot(_unpack(vA[:, _ds(k * T, T)]), p)
                store_o(g, lax.fori_loop(0, NT, pv, jnp.zeros((32, GW), F32)))
                return c
            lax.fori_loop(0, NG, group, 0)
            run(out_items(t, woAT) + ln_items(t) + proj_b_items(t))
            return c

        def b_tile(t, r):
            a = lax.broadcasted_iota(I32, (3 * T, T), 0) + (t * T - WIN)
            b = lax.broadcasted_iota(I32, (3 * T, T), 1) + t * T
            valid = (a >= 0) & (a <= b) & (b - a < WIN)

            def group(g, c):
                qg = _unpack(qB[_ds(g * (GR // 2), GR // 2, 8), _ds(t * T, T)]).astype(F32)
                k = _unpack(kB[g, _ds(t * (T // 2), 3 * T // 2, 64), 0:GR])
                head = lax.broadcasted_iota(I32, (GR, T), 0) // DH
                outs = []
                for j in range(HG):
                    s = jnp.where(valid, _dot(k, jnp.where(head == j, qg, 0.0).astype(BF16)), NEG)
                    p = jnp.exp2(s - jnp.max(s, axis=0, keepdims=True)).astype(BF16)
                    outs.append(_dot(_unpack(vB[_ds((g * HG + j) * 16, 16, 16), _ds(t * T, 3 * T)]), p))
                store_o(g, jnp.concatenate(outs, axis=1))
                return c
            lax.fori_loop(0, NG, group, 0)
            run(out_items(t, woBT))

            @pl.when(r == 0)
            def _():
                run(ln_items(t) + proj_a_items(t))
            return r

        def pair(r, c):
            lax.fori_loop(0, NT, a_tile, 0)
            lax.fori_loop(0, NT, b_tile, r)
            return c
        lax.fori_loop(0, 2, pair, 0)

        def emit(t, c):
            out_st[:, _ds(t * T, T)] = xres[:, _ds(t * T, T)].astype(BF16)
            return c
        lax.fori_loop(0, NT, emit, 0)
        cp = pltpu.make_async_copy(out_st, out_hbm, out_sem.at[0])
        cp.start()
        cp.wait()


OPW = H * T + (NV // 16) * 8 * 256 + 128


@jax.jit
def pallas_interleave_layers__grouped_kv_mqa__sliding_block__prompt_kernel(A_x, A_wq, A_wk, A_wv, A_wo, B_x, B_wqkv, B_wo):
    del B_x
    xT = jnp.swapaxes(A_x[0], 0, 1)
    outT = pl.pallas_call(
        kernel,
        out_shape=jax.ShapeDtypeStruct((D, S), BF16),
        in_specs=[pl.BlockSpec(memory_space=pl.ANY)] * 7,
        out_specs=pl.BlockSpec(memory_space=pl.ANY),
        scratch_shapes=[
            pltpu.VMEM((D, S), BF16),
            pltpu.VMEM((D, D), BF16),
            pltpu.VMEM((DH, D), BF16),
            pltpu.VMEM((DH, D), BF16),
            pltpu.VMEM((D, D), BF16),
            pltpu.VMEM((D, 3 * D), BF16),
            pltpu.VMEM((D, D), BF16),
            pltpu.VMEM((D, S), BF16),
            pltpu.SemaphoreType.DMA((XC + 6,)),
            pltpu.SemaphoreType.DMA((1,)),
            pltpu.VMEM((D, S), F32),
            pltpu.VMEM((D // 2, T), I32),
            pltpu.VMEM((D // 2 + 32, D), I32),
            pltpu.VMEM((D // 2, D), I32),
            pltpu.VMEM((3 * D // 2, D), I32),
            pltpu.VMEM((D // 2, D), I32),
            pltpu.VMEM((S // 2, H * T), I32),
            pltpu.VMEM((NG, 4, BAND // 2, 128), I32),
            pltpu.VMEM((D // 2, T), I32),
            pltpu.VMEM((24, 128), F32),
            pltpu.VMEM((6, GR // 2, 128), I32),
            pltpu.VMEM((16, H * S), I32),
            pltpu.VMEM((32, H * S), F32),
            pltpu.VMEM((S // 2, 32), I32),
            pltpu.VMEM((16, S), I32),
            pltpu.VMEM((D // 2, S), I32),
            pltpu.VMEM((NG, (S + WIN) // 2, 128), I32),
            pltpu.VMEM((NG, 4, (S + 160) // 2, 128), I32),
            pltpu.VMEM((H * 16, S + WIN), I32),
            pltpu.VMEM((S, GW), F32),
        ] + [pltpu.VMEM((8, OPW), F32)] * 4,
        compiler_params=pltpu.CompilerParams(vmem_limit_bytes=100 * 1024 * 1024),
        name="fused_layers",
    )(xT, A_wq, A_wk.T, A_wv.T, A_wo, B_wqkv, B_wo)
    return jnp.swapaxes(outT, 0, 1)[None]
```

```python
import math

import jax
import jax.numpy as jnp
from jax import lax
import jax.experimental.pallas as pl
import jax.experimental.pallas.tpu as pltpu

S, D, H, DH, WIN = 2048, 448, 16, 28, 256
T = 128
NT = S // T
HG = 4
NG = H // HG
GR = HG * DH
GW = HG * T
BAND = WIN + 32
NV = 256
NV_FIRST = 192
X_FIRST, X_SPLIT = 2, 7
QSCALE = (DH ** -0.5) * math.log2(math.e)
NEG = -1e30
L_MIN, L_MAX = 2.0 ** -60, 2.0 ** 100
F32, BF16, I32 = jnp.float32, jnp.bfloat16, jnp.int32

D_ORDER = [0, 1, 8, 9, 2, 3, 10, 11, 4, 5, 12, 13, 6, 7]
D_SLOT = {d: (d // 8 + 2 * (d // 2 % 2), d % 2 + 2 * (d % 8 // 4)) for d in range(DH // 2)}
QW = NG * 7 * 2 * T
OPW = QW + ((NV // 32) * 7 * 4 + 2) * T


def _dot(a, b):
    return jnp.dot(a, b, preferred_element_type=F32)


def _pack(x):
    r, c = x.shape
    if c > 128:
        return pltpu.bitcast(x.astype(BF16), I32)
    half = max(32, -(-r // 32) * 16)
    if 2 * half > r:
        x = jnp.concatenate([x, jnp.zeros((2 * half - r, c), x.dtype)], axis=0)
    w = pltpu.bitcast(jnp.concatenate([x[:half], x[half:]], axis=1).astype(BF16), I32)
    return jnp.concatenate([w[:, :c], w[:, c:]], axis=0)[:r // 2]


def _unpack(x):
    return pltpu.bitcast(x, BF16)


def _tree(op, xs):
    xs = list(xs)
    while len(xs) > 1:
        xs = [op(xs[i], xs[i + 1]) if i + 1 < len(xs) else xs[i] for i in range(0, len(xs), 2)]
    return xs[0]


def _ds(start, size, mult=T):
    if isinstance(start, int):
        return pl.ds(start, size)
    return pl.ds(pl.multiple_of(start, mult), size)


def _zip_in(main, extra):
    out = []
    for n, it in enumerate(main):
        out.append(it)
        out += extra[len(extra) * n // len(main):len(extra) * (n + 1) // len(main)]
    return out


def _lane_bit(width, bit):
    return ((lax.broadcasted_iota(I32, (8, 128), 1) // width) & bit) != 0


def _pick(mask, a, b):
    r = a.shape[0]
    return jnp.where(mask[None], a.reshape(r // 8, 8, 128), b.reshape(r // 8, 8, 128)).reshape(r, 128)


def _halves(y):
    z = jnp.zeros((2, T), F32)
    return jnp.concatenate([y[0:DH // 2], z, y[DH // 2:DH], z], axis=0)


def _kernel(x_hbm, wq_hbm, wk_hbm, wv_hbm, woA_hbm, wqkv_hbm, woB_hbm, out_hbm,
            x_in, wq_in, wk_in, wv_in, woA_in, wqkv_in, woB_in, out_st, in_sem, out_sem, bar_sem,
            xres, xnA, xnB, wA, woAT, wB, woBT, pA, pB, pY, oA, oB, chk, qmask,
            qA, kA0, vA0, kA1, vA1, qB, kB, vB, sX, *rest_refs):
    ops, kY = rest_refs[0:4], rest_refs[4:8]
    x_cp = [pltpu.make_async_copy(x_hbm.at[:, pl.ds(a * T, (b - a) * T)], x_in.at[:, pl.ds(a * T, (b - a) * T)],
                                  in_sem.at[i])
            for i, (a, b) in enumerate(((0, X_FIRST), (X_FIRST, X_SPLIT), (X_SPLIT, NT)))]
    w_cp = [pltpu.make_async_copy(src, dst, in_sem.at[3 + i]) for i, (src, dst) in enumerate(
        ((wk_hbm, wk_in), (wv_hbm, wv_in), (wq_hbm, wq_in), (woA_hbm, woA_in), (wqkv_hbm, wqkv_in),
         (woB_hbm, woB_in)))]
    for c in (w_cp[0], w_cp[1], x_cp[0], w_cp[2], *x_cp[1:], *w_cp[3:]):
        c.start()

    def out_copy(t):
        return pltpu.make_async_copy(out_st.at[:, _ds(t * T, T)], out_hbm.at[:, _ds(t * T, T)], out_sem.at[0])

    pacer = {"side": [], "done": 0, "time": 0.0, "total": 1.0, "gate": 0, "v": None, "slot": None}

    def tick(y, cycles, weight):
        n = max(1, cycles // 8)
        for a in range(n):
            pacer["v"] = (y, a * y.shape[0] // n // 8 * 8)
            side = pacer["side"]
            if side and pacer["gate"] < side[0][0]:
                pacer["total"] -= weight * cycles / n
                continue
            pacer["time"] += weight * cycles / n
            want = min(len(side), int(len(side) * pacer["time"] / pacer["total"]))
            while pacer["done"] < want and pacer["gate"] >= side[pacer["done"]][0]:
                side[pacer["done"]][1]()
                pacer["done"] += 1

    def pace(buf):
        if pacer["v"] is not None:
            y, r = pacer["v"]
            buf[0:8, pacer["slot"]] = y[r:r + 8, 0:T]

    def drain():
        while pacer["done"] < len(pacer["side"]):
            pacer["side"][pacer["done"]][1]()
            pacer["done"] += 1

    def run(items, side=(), tail=0):
        pacer.update(side=list(side), done=0, time=0.0, total=max(1.0, sum(c for c, _ in items) - tail),
                     gate=0, v=None)
        for _, fn in items:
            fn()
        drain()
        pacer.update(side=[], done=0)

    def fence():
        pl.semaphore_signal(bar_sem, 1)
        pl.semaphore_wait(bar_sem, 1)

    def wdot(w_ref, r0, n, x_ref):
        y = _dot(_unpack(w_ref[pl.ds(r0 // 2, n // 2), :]), _unpack(x_ref[...]))
        tick(y, n, 0.0)
        return y

    def ln_stats(st, x, first):
        if first:
            st["c"] = jnp.broadcast_to(x[0:1], (8, T))
        d = [x[i:i + 8] - st["c"] for i in range(0, x.shape[0], 8)]
        s1, s2 = _tree(jnp.add, d), _tree(jnp.add, [v * v for v in d])
        st["s1"] = s1 if first else st["s1"] + s1
        st["s2"] = s2 if first else st["s2"] + s2

    def ln_items(t, xn, st, zero, src):
        def norm():
            e1 = jnp.sum(st["s1"], axis=0, keepdims=True) * (1.0 / D)
            e2 = jnp.sum(st["s2"], axis=0, keepdims=True) * (1.0 / D)
            r = lax.rsqrt(jnp.maximum(e2 - e1 * e1, 0.0) + 1e-5)
            xn[...] = _pack((src[:, _ds(t * T + zero, T)].astype(F32) - (st["c"][0:1] + e1)) * r)
        return [(0, norm)]

    def input_norm_items(t, xn, zero):
        st = {}

        def stats():
            for g in range(NG):
                ln_stats(st, x_in[pl.ds(g * GR, GR), _ds(t * T, T)].astype(F32), g == 0)
        return [(0, stats)] + ln_items(t, xn, st, zero, x_in)

    def proj_a_items(t, kA, vA, xn):
        def kv():
            y = wdot(wA, D, 64, xn)
            kT = jnp.concatenate([_halves(y[0:DH]), jnp.zeros((96, T), F32)], axis=0)
            kA[_ds(t * (T // 2), T // 2, T // 2), :] = _pack(kT.T)[:, 0:32]
            vA[:, _ds(t * T, T)] = _pack(jnp.concatenate([y[DH:2 * DH], jnp.ones((4, T), F32)], axis=0))

        def q(g):
            def f():
                y = wdot(wA, g * GR, GR, xn) * QSCALE
                qA[:, _ds(t * (H * T) + g * GW, GW)] = _pack(
                    jnp.concatenate([_halves(y[j * DH:(j + 1) * DH]) for j in range(HG)], axis=1))
            return f
        return [(0, kv)] + [(0, q(g)) for g in range(NG)]

    def key_factor_items(kA):
        def one(kb, d):
            def f():
                k = _unpack(kA[pl.ds(kb * 16, 16), :]).astype(F32)
                lo = jnp.broadcast_to(k[:, d:d + 1], (32, 128))
                hi = jnp.broadcast_to(k[:, d + 16:d + 17], (32, 128))
                a11, a12, a21, a22 = lo[0:16], hi[0:16], lo[16:32], hi[16:32]
                s1 = a21 + a22
                s2 = s1 - a11
                b, slot = D_SLOT[d]
                for p, v in enumerate((a11, a12, a12 - s2, a22, s1, s2, a11 - a21)):
                    ops[b][:, pl.ds(QW + ((kb * 7 + p) * 4 + slot) * T, T)] = v
            return (0, f)
        return [one(kb, d) for kb in range(NV // 32) for d in D_ORDER]

    def query_factor_items(t):
        def one(g, b):
            def f():
                q, r0 = _unpack(qA[:, _ds(t * (H * T) + g * GW, GW)]).astype(F32), b % 2 * 8
                lo, hi = q[r0:r0 + 8], q[16 + r0:24 + r0]
                b11, b12, b21, b22 = lo[:, 0:256], lo[:, 256:512], hi[:, 0:256], hi[:, 256:512]
                t1 = b12 - b11
                t2 = b22 - t1
                pace(ops[b])
                for p, v in enumerate((b11, b21, b22, b21 - t2, t1, t2, b22 - b12)):
                    ops[b][0:8, pl.ds((g * 7 + p) * 2 * T, 2 * T)] = v
            return (0, f)
        return [one(g, b) for g in range(NG) for b in range(4)]

    def proj_b_items(t):
        def k(g):
            def f():
                y = wdot(wB, D + g * GR, GR, xnA)
                cur = _pack(jnp.concatenate([y, jnp.zeros((128 - GR, T), F32)], axis=0).T)
                kB[g, _ds(t * (T // 2) + WIN // 2, T // 2, T // 2), :] = cur
                w = jnp.concatenate([kB[g, _ds(t * (T // 2) + (WIN - 96) // 2, 48, 16), :], cur], axis=0)
                b0, b1 = _lane_bit(DH, 1), _lane_bit(DH, 2)
                z = [_pick(b0, w[16:112], w[0:96]), _pick(b0, w[0:96], w[16:112])]
                rows = _ds(t * (T // 2) + 80, T // 2, 16)
                for a in range(2):
                    kY[g][a, rows, :] = _pick(b1, z[a][32:96], z[a][0:64])
                    kY[g][a + 2, rows, :] = _pick(b1, z[a][0:64], z[a][32:96])
            return f

        def q(g):
            def f():
                qB[pl.ds(g * GR // 2, GR // 2), _ds(t * T, T)] = _pack(wdot(wB, g * GR, GR, xnA) * QSCALE)
            return f

        def v(g):
            def f():
                y = wdot(wB, 2 * D + g * GR, GR, xnA)
                ones = jnp.ones((4, T), F32)
                parts = []
                for j in range(HG):
                    parts += [y[j * DH:(j + 1) * DH], ones]
                vB[pl.ds(g * 64, 64), _ds(t * T + WIN, T)] = _pack(jnp.concatenate(parts, axis=0))
            return f
        return [(0, f(g)) for f in (k, q, v) for g in range(NG)]

    def out_items(t, woT, o_ref, st, src):
        def part(g):
            def f():
                rows, cols = pl.ds(g * GR, GR), _ds(t * T, T)
                x = src[rows, cols].astype(F32) + wdot(woT, g * GR, GR, o_ref)
                if st is None:
                    out_st[rows, cols] = x.astype(BF16)
                else:
                    xres[rows, cols] = x
                    ln_stats(st, x, g == 0)
            return (0, f)
        items = [part(g) for g in range(NG)]
        if st is None:
            items.append((0, lambda: out_copy(t).start()))
        return items

    def store_o(o_ref, g, acc):
        on = acc[0:DH] * pl.reciprocal(acc[DH:DH + 1])
        o_ref[_ds(g * (GR // 2), GR // 2, 8), :] = _pack(
            jnp.concatenate([on[:, j * T:(j + 1) * T] for j in range(HG)], axis=0))

    def finish_group(o_ref, g, acc):
        store_o(o_ref, g, acc)
        den = [acc[24:32, j * T:(j + 1) * T] for j in range(HG)]
        chk[0:8] = chk[0:8] + _tree(jnp.add, [acc[i:i + 8, j * T:(j + 1) * T]
                                              for i in range(0, 32, 8) for j in range(HG)])
        chk[8:16] = jnp.minimum(chk[8:16], _tree(jnp.minimum, den))
        chk[16:24] = jnp.maximum(chk[16:24], _tree(jnp.maximum, den))

    def attn_a_items(t, kA, vA, do_qk, do_pv, nv, restage=()):
        st = {}
        steps = [(g, c) for g in range(NG) for c in range(NT)]
        bound = [nv + (S - nv) * i // NT // 16 * 16 for i in range(NT + 1)]

        def pv(n):
            def f():
                g, c = steps[n]
                p = _unpack(pA[pl.ds(c * (T // 2), T // 2), pl.ds(g * GW, GW)])
                o = _dot(_unpack(vA[:, pl.ds(c * T, T)]), p)
                st["acc"] = o if c == 0 else st["acc"] + o
                pacer["gate"] = n + 1
                tick(o, 32, 1.0)
                if c == NT - 1:
                    finish_group(oA, g, st["acc"])
            return (32, f)

        def qk(n):
            g, c = steps[n]
            lo, hi = bound[c], bound[c + 1]

            def f():
                if c == 0:
                    st["q"] = _unpack(qA[:, _ds(t * (H * T) + g * GW, GW)])
                rows = pl.ds(lo // 2, (hi - lo) // 2)
                s = _dot(_unpack(kA[rows, :]), st["q"])
                pA[rows, pl.ds(g * GW, GW)] = _pack(jnp.exp2(s))
                tick(s, hi - lo, 1.0)
            return (hi - lo, f)

        def vpu_block(g, kb):
            m = {}

            def emit(r, c, s):
                pA[pl.ds(kb * 16 + r * 8, 8), pl.ds(g * GW + c * 2 * T, 2 * T)] = _pack(
                    jnp.exp2(jnp.concatenate(s, axis=1)))

            def product(p, dst, init=None, then=None):
                def one(n, d):
                    def f():
                        b, slot = D_SLOT[d]
                        if n % 2 == 0:
                            pace(ops[b])
                        kk = ops[b][:, pl.ds(QW + ((kb * 7 + p) * 4 + slot) * T, T)]
                        term = [kk * ops[b][d % 8:d % 8 + 1, pl.ds(((g * 7 + p) * 2 + j) * T, T)] for j in range(2)]
                        base = m[dst] if n else m.get(init)
                        m[dst] = term if base is None else [x + y for x, y in zip(base, term)]
                        if n == DH // 2 - 1 and then:
                            then()
                    return f
                return [one(n, d) for n, d in enumerate(D_ORDER)]

            def mix():
                emit(1, 1, [x + y for x, y in zip(m["u3"], m["m5"])])
                m["u4"] = [x + y for x, y in zip(m["u2"], m["m5"])]
            return (product(0, "m1") + product(1, "c11", "m1", lambda: emit(0, 0, m["c11"]))
                    + product(5, "u2", "m1") + product(6, "u3", "u2") + product(4, "m5", None, mix)
                    + product(2, "c12", "u4", lambda: emit(0, 1, m["c12"]))
                    + product(3, "c21", "u3", lambda: emit(1, 0, m["c21"])))

        if not do_qk:
            return [pv(n) for n in range(len(steps))], []
        ahead = -(-nv // T) if do_pv else 0
        side = []
        for g in range(NG):
            fs = [f for kb in range(nv // 32) for f in vpu_block(g, kb)] + [f for _, f in restage[4 * g:4 * g + 4]]
            side += [(g * NT + ahead if do_pv else 0, f) for f in fs]
        items = [pv(n) for n in range(ahead)]
        for n in range(len(steps)):
            if do_pv and n + ahead < len(steps):
                items.append(pv(n + ahead))
            items.append(qk(n))
        return items, side

    def attn_b_items(t, qk_b0=0, pv_c0=0):
        def qk(g):
            def f():
                qg = qB[pl.ds(g * GR // 2, GR // 2), _ds(t * T, T)]
                r0 = qk_b0 * 16
                n = BAND // 2 - r0
                for u in range(4):
                    s = _dot(_unpack(kY[g][u, _ds(t * (T // 2) + r0, n, 16), 0:GR]), _unpack(qg & qmask[u]))
                    e = jnp.exp2(s)
                    if r0:
                        e = jnp.concatenate([jnp.zeros((2 * r0, T), F32), e], axis=0)
                    pB[pl.ds((g * 4 + u) * (BAND // 4), BAND // 4), :] = _pack(
                        jnp.concatenate([e[:BAND // 2], e[BAND // 2:]], axis=1))
                tick(s, 2 * n, 0.0)
            return (0, f)

        def unskew(g):
            def f():
                odd, high = _lane_bit(32, 1), _lane_bit(32, 2)
                zb = jnp.zeros((16, 128), I32)

                def band(u):
                    w = pB[pl.ds((g * 4 + u) * (BAND // 4), BAND // 4), :]
                    return jnp.concatenate([w[0:16, 0:T] & qmask[4, 0:16], w[16:, 0:T], w[:-16, T:],
                                            w[-16:, T:] & qmask[5, 0:16]], axis=0)
                for a in range(2):
                    mid = {b: _pick(odd, jnp.concatenate([zb, band(b ^ 1)], axis=0),
                                    jnp.concatenate([band(b), zb], axis=0)) for b in (a, a + 2)}
                    for h in (a, a + 2):
                        pY[g, h] = _pick(high, jnp.concatenate([zb, zb, mid[h ^ 2]], axis=0),
                                         jnp.concatenate([mid[h], zb, zb], axis=0))
            return (0, f)

        def pv(g):
            def f():
                outs = []
                for h in range(HG):
                    v = vB[pl.ds((g * HG + h) * 16, 16), _ds((t + pv_c0) * T, (3 - pv_c0) * T)]
                    outs.append(_dot(_unpack(v), _unpack(pY[g, h, pv_c0 * 64:3 * T // 2, :])))
                tick(outs[0], 32 * (3 - pv_c0), 0.0)
                finish_group(oB, g, jnp.concatenate(outs, axis=1))
            return (0, f)
        return [[qk(g), unskew(g)] for g in range(NG)], [[pv(g)] for g in range(NG)]

    def post_a(t, src, zero):
        st = {}
        return out_items(t, woAT, oA, st, src), ln_items(t, xnA, st, zero, xres), proj_b_items(t)

    def post_b(t, last, zero):
        if last:
            return out_items(t, woBT, oB, None, xres), [], []
        st = {}
        return (out_items(t, woBT, oB, st, xres), ln_items(t, xnB, st, zero, xres),
                proj_a_items(t, kA1, vA1, xnB))

    def window(pa, qk, pv):
        return (pa[:8] + qk[0] + pa[8:9] + qk[1] + pa[9:10] + qk[2] + pa[10:11] + qk[3]
                + pv[0] + pv[1] + pv[2] + pa[11:])

    def layer_pair(r, zero0, under_first):
        kA, vA = (kA0, vA0) if r == 0 else (kA1, vA1)
        src, last = (x_in, False) if r == 0 else (xres, True)
        done = [(0, drain)]
        pacer["slot"] = _ds(zero0 + (OPW - T), T)

        main, side = attn_a_items(0, kA, vA, True, False, NV_FIRST, query_factor_items(1))
        run(under_first(main), side, 100)
        fence()

        main, side = attn_a_items(1, kA, vA, True, True, NV)
        oa, la, pa = post_a(0, src, zero0)
        qk, pv = attn_b_items(0, 5, 2)
        rest = pa[:8] + qk[0] + qk[1] + qk[2] + qk[3] + pa[8:] + pv[0] + pv[1] + pv[2]
        run(main[:-2] + oa + la + main[-2:] + _zip_in(rest, done + query_factor_items(2)), side)
        fence()

        def body(j, carry):
            i, zero = j + 2, (j >> 20) * T
            pacer["slot"] = _ds(zero + (OPW - T), T)
            main, side = attn_a_items(i, kA, vA, True, True, NV)
            oa, la, pa = post_a(i - 1, src, zero)
            ob, lb, pb = post_b(i - 2, last, zero)
            qk, pv = attn_b_items(i - 1)
            sq = query_factor_items(jnp.minimum(i + 1, NT - 1))
            late = attn_b_items(i - 2)[1][3]
            run(main + done + _zip_in(late + oa + la + ob, sq) + lb + window(pa, qk, pv) + pb, side, 30)
            return carry
        lax.fori_loop(0, NT - 2, body, 0)

        pacer["slot"] = _ds(zero0 + (OPW - T), T)
        main, _ = attn_a_items(None, kA, vA, False, True, NV)
        if not last:
            fence()
            run(_zip_in(main, query_factor_items(0) + key_factor_items(kA1)))
            fence()
            main = []
        oa, la, pa = post_a(NT - 1, src, zero0)
        ob, lb, pb = post_b(NT - 2, last, zero0)
        qk, pv = attn_b_items(NT - 1)
        late = attn_b_items(NT - 2)[1][3]
        run(main + late + oa + la + ob + lb + window(pa, qk, pv) + pb)
        return (pv[3],) + post_b(NT - 1, last, zero0)

    row = lax.broadcasted_iota(I32, (GR // 2, 128), 0)
    lane = lax.broadcasted_iota(I32, (GR // 2, 128), 1)
    for u in range(4):
        qmask[u] = jnp.where(((row // (DH // 2)) ^ (lane // 32)) == u, -1, 0)
    lo_w, hi_w = 0xFFFF, -0x10000
    qmask[4] = jnp.where(2 * row > lane % 32, lo_w, 0) | jnp.where(2 * row + 1 > lane % 32, hi_w, 0)
    qmask[5] = jnp.where(2 * row <= lane % 32, lo_w, 0) | jnp.where(2 * row + 1 <= lane % 32, hi_w, 0)
    chk[0:8] = jnp.zeros((8, 128), F32)
    chk[8:24] = jnp.ones((16, 128), F32)
    for g in range(NG):
        kB[g, 0:WIN // 2, :] = jnp.zeros((WIN // 2, 128), I32)
        kY[g][:, 0:80, :] = jnp.zeros((4, 80, 128), I32)
    vB[:, 0:WIN] = jnp.zeros((H * 16, WIN), I32)

    w_cp[0].wait()
    w_cp[1].wait()
    wA[D // 2:D // 2 + 32, :] = _pack(jnp.concatenate(
        [wk_in[...].astype(F32), wv_in[...].astype(F32), jnp.zeros((8, D), F32)], axis=0))
    zero0 = jnp.max(chk[0:8]).astype(I32) * T
    pacer["slot"] = _ds(zero0 + (OPW - T), T)

    def transpose_item(src, dst, i):
        def f():
            dst[pl.ds(i * D // 2, D // 2), :] = _pack(src[:, i * D:(i + 1) * D].T)
        return (0, f)

    def first_tiles(t0, t1):
        items = []
        for t in range(t0, t1):
            cur, nxt = (xnB, xnA) if t % 2 == 0 else (xnA, xnB)
            if t + 1 < NT:
                items += input_norm_items(t + 1, nxt, zero0)
            items += proj_a_items(t, kA0, vA0, cur)
        return items

    x_cp[0].wait()
    run(input_norm_items(0, xnB, zero0))
    w_cp[2].wait()
    run([transpose_item(wq_in, wA, 0)])
    run(first_tiles(0, X_FIRST - 1))
    x_cp[1].wait()
    run(first_tiles(X_FIRST - 1, X_SPLIT - 1))
    x_cp[2].wait()
    fence()
    run(_zip_in(first_tiles(X_SPLIT - 1, NT), query_factor_items(0) + key_factor_items(kA0)))
    fence()
    for c in w_cp[3:]:
        c.wait()
    weights = ([transpose_item(woA_in, woAT, 0)] + [transpose_item(wqkv_in, wB, i) for i in range(3)]
               + [transpose_item(woB_in, woBT, 0)])

    late, ob, lb, pb = layer_pair(0, zero0, lambda main: _zip_in(main, weights))
    late, ob, _, _ = layer_pair(1, zero0, lambda main: late + main[0:1] + ob + lb + main[1:4] + pb + main[4:])
    run(late + ob)
    for t in range(NT):
        out_copy(t).wait()

    sub = lax.broadcasted_iota(I32, (8, 128), 0)
    ok = (jnp.abs(chk[0:8]) < float("inf")) & (((chk[8:16] >= L_MIN) & (chk[16:24] <= L_MAX)) | (sub < 4))

    @pl.when(jnp.min(jnp.where(ok, 1.0, 0.0)) < 0.5)
    def _():
        def first(t, c):
            xres[:, _ds(t * T, T)] = x_in[:, _ds(t * T, T)].astype(F32)
            run(input_norm_items(t, xnB, 0) + proj_a_items(t, kA0, vA0, xnB))
            return c
        lax.fori_loop(0, NT, first, 0)

        def a_tile(t, c):
            def group(g, c):
                q = _unpack(qA[:, _ds(t * (H * T) + g * GW, GW)])

                def scores(k, m):
                    s = _dot(_unpack(kA0[_ds(k * 64, 64, 64), :]), q)
                    sX[_ds(k * T, T), :] = s
                    return jnp.maximum(m, jnp.max(s, axis=0, keepdims=True))
                m = lax.fori_loop(0, NT, scores, jnp.full((1, GW), -jnp.inf, F32))

                def weighted(k, acc):
                    p = jnp.exp2(sX[_ds(k * T, T), :] - m).astype(BF16)
                    return acc + _dot(_unpack(vA0[:, _ds(k * T, T)]), p)
                store_o(oA, g, lax.fori_loop(0, NT, weighted, jnp.zeros((32, GW), F32)))
                return c
            lax.fori_loop(0, NG, group, 0)
            oa, la, pa = post_a(t, xres, 0)
            run(oa + la + pa)
            return c

        def b_tile(t, r):
            key = lax.broadcasted_iota(I32, (3 * T, T), 0) + (t * T - WIN)
            query = lax.broadcasted_iota(I32, (3 * T, T), 1) + t * T
            valid = (key >= 0) & (key <= query) & (query - key < WIN)

            def group(g, c):
                qg = _unpack(qB[_ds(g * (GR // 2), GR // 2, 8), _ds(t * T, T)]).astype(F32)
                k = _unpack(kB[g, _ds(t * (T // 2), 3 * T // 2, 64), 0:GR])
                head = lax.broadcasted_iota(I32, (GR, T), 0) // DH
                outs = []
                for j in range(HG):
                    s = jnp.where(valid, _dot(k, jnp.where(head == j, qg, 0.0).astype(BF16)), NEG)
                    p = jnp.exp2(s - jnp.max(s, axis=0, keepdims=True)).astype(BF16)
                    outs.append(_dot(_unpack(vB[_ds((g * HG + j) * 16, 16, 16), _ds(t * T, 3 * T)]), p))
                store_o(oB, g, jnp.concatenate(outs, axis=1))
                return c
            lax.fori_loop(0, NG, group, 0)
            st = {}
            run(out_items(t, woBT, oB, st, xres))

            @pl.when(r == 0)
            def _():
                run(ln_items(t, xnB, st, 0, xres) + proj_a_items(t, kA0, vA0, xnB))
            return r

        def pair(r, c):
            lax.fori_loop(0, NT, a_tile, 0)
            lax.fori_loop(0, NT, b_tile, r)
            return c
        lax.fori_loop(0, 2, pair, 0)

        def emit(t, c):
            out_st[:, _ds(t * T, T)] = xres[:, _ds(t * T, T)].astype(BF16)
            return c
        lax.fori_loop(0, NT, emit, 0)
        cp = pltpu.make_async_copy(out_st, out_hbm, out_sem.at[0])
        cp.start()
        cp.wait()


@jax.jit
def pallas_interleave_layers__grouped_kv_mqa__sliding_block__prompt_kernel(
        A_x, A_wq, A_wk, A_wv, A_wo, B_x, B_wqkv, B_wo):
    del B_x
    out_t = pl.pallas_call(
        _kernel,
        out_shape=jax.ShapeDtypeStruct((D, S), BF16),
        in_specs=[pl.BlockSpec(memory_space=pl.ANY)] * 7,
        out_specs=pl.BlockSpec(memory_space=pl.ANY),
        scratch_shapes=[
            pltpu.VMEM((D, S), BF16),
            pltpu.VMEM((D, D), BF16),
            pltpu.VMEM((DH, D), BF16),
            pltpu.VMEM((DH, D), BF16),
            pltpu.VMEM((D, D), BF16),
            pltpu.VMEM((D, 3 * D), BF16),
            pltpu.VMEM((D, D), BF16),
            pltpu.VMEM((D, S), BF16),
            pltpu.SemaphoreType.DMA((9,)),
            pltpu.SemaphoreType.DMA((1,)),
            pltpu.SemaphoreType.REGULAR,
            pltpu.VMEM((D, S), F32),
            pltpu.VMEM((D // 2, T), I32),
            pltpu.VMEM((D // 2, T), I32),
            pltpu.VMEM((D // 2 + 32, D), I32),
            pltpu.VMEM((D // 2, D), I32),
            pltpu.VMEM((3 * D // 2, D), I32),
            pltpu.VMEM((D // 2, D), I32),
            pltpu.VMEM((S // 2, H * T), I32),
            pltpu.VMEM((NG * BAND, 2 * T), I32),
            pltpu.VMEM((NG, HG, 3 * T // 2, 128), I32),
            pltpu.VMEM((D // 2, T), I32),
            pltpu.VMEM((D // 2, T), I32),
            pltpu.VMEM((24, 128), F32),
            pltpu.VMEM((6, GR // 2, 128), I32),
            pltpu.VMEM((16, H * S), I32),
            pltpu.VMEM((S // 2, 32), I32),
            pltpu.VMEM((16, S), I32),
            pltpu.VMEM((S // 2, 32), I32),
            pltpu.VMEM((16, S), I32),
            pltpu.VMEM((D // 2, S), I32),
            pltpu.VMEM((NG, (S + WIN) // 2, 128), I32),
            pltpu.VMEM((H * 16, S + WIN), I32),
            pltpu.VMEM((S, GW), F32),
        ] + [pltpu.VMEM((16, OPW), F32)] * 4
          + [pltpu.VMEM((4, (S + 160) // 2, 128), I32)] * NG,
        compiler_params=pltpu.CompilerParams(vmem_limit_bytes=100 * 1024 * 1024),
        name="fused_layers",
    )(jnp.swapaxes(A_x[0], 0, 1), A_wq, A_wk.T, A_wv.T, A_wo, B_wqkv, B_wo)
    return jnp.swapaxes(out_t, 0, 1)[None]
```

```python
import math

import jax
import jax.numpy as jnp
from jax import lax
import jax.experimental.pallas as pl
import jax.experimental.pallas.tpu as pltpu

S, D, H, DH, WIN = 2048, 448, 16, 28, 256
T = 128
NT = S // T
HG = 4
NG = H // HG
GR = HG * DH
GW = HG * T
BAND = WIN + 32
NV = 256
NV_FIRST = 192
X_FIRST, X_SPLIT = 2, 8
QSCALE = (DH ** -0.5) * math.log2(math.e)
NEG = -1e30
L_MIN, L_MAX = 2.0 ** -40, 2.0 ** 100
F32, BF16, I32 = jnp.float32, jnp.bfloat16, jnp.int32

D_ORDER = [0, 1, 8, 9, 2, 3, 10, 11, 4, 5, 12, 13, 6, 7]
D_SLOT = {d: (d // 8 + 2 * (d // 2 % 2), d % 2 + 2 * (d % 8 // 4)) for d in range(DH // 2)}
QW = NG * 7 * 2 * T
OPW = QW + ((NV // 32) * 7 * 4 + 3) * T


def _dot(a, b):
    return jnp.dot(a, b, preferred_element_type=F32)


def _pack(x):
    r, c = x.shape
    if c > 128:
        return pltpu.bitcast(x.astype(BF16), I32)
    half = max(32, -(-r // 32) * 16)
    if 2 * half > r:
        x = jnp.concatenate([x, jnp.zeros((2 * half - r, c), x.dtype)], axis=0)
    w = pltpu.bitcast(jnp.concatenate([x[:half], x[half:]], axis=1).astype(BF16), I32)
    return jnp.concatenate([w[:, :c], w[:, c:]], axis=0)[:r // 2]


def _unpack(x):
    return pltpu.bitcast(x, BF16)


def _tree(op, xs):
    xs = list(xs)
    while len(xs) > 1:
        xs = [op(xs[i], xs[i + 1]) if i + 1 < len(xs) else xs[i] for i in range(0, len(xs), 2)]
    return xs[0]


def _ds(start, size, mult=T):
    if isinstance(start, int):
        return pl.ds(start, size)
    return pl.ds(pl.multiple_of(start, mult), size)


def _zip_in(main, extra):
    out = []
    for n, it in enumerate(main):
        out.append(it)
        out += extra[len(extra) * n // len(main):len(extra) * (n + 1) // len(main)]
    return out


def _lane_bit(width, bit):
    return ((lax.broadcasted_iota(I32, (8, 128), 1) // width) & bit) != 0


def _pick(mask, a, b):
    r = a.shape[0]
    return jnp.where(mask[None], a.reshape(r // 8, 8, 128), b.reshape(r // 8, 8, 128)).reshape(r, 128)


def _halves(y):
    z = jnp.zeros((2, T), F32)
    return jnp.concatenate([y[0:DH // 2], z, y[DH // 2:DH], z], axis=0)


def _kernel(x_hbm, wq_hbm, wk_hbm, wv_hbm, woA_hbm, wqkv_hbm, woB_hbm, out_hbm,
            x_in, wq_in, wk_in, wv_in, woA_in, wqkv_in, woB_in, out_st, in_sem, out_sem, bar_sem,
            xres, xnA, xnB, wA, woAT, wB, woBT, pA, pB, pY, oA, oB, chk, qmask,
            qA, kA0, vA0, kA1, vA1, qB, kB, vB, sX, *rest_refs):
    ops, kY = rest_refs[0:4], rest_refs[4:8]
    x_cp = [pltpu.make_async_copy(x_hbm.at[:, pl.ds(a * T, (b - a) * T)], x_in.at[:, pl.ds(a * T, (b - a) * T)],
                                  in_sem.at[i])
            for i, (a, b) in enumerate(((0, X_FIRST), (X_FIRST, X_SPLIT), (X_SPLIT, NT)))]
    w_cp = [pltpu.make_async_copy(src, dst, in_sem.at[3 + i]) for i, (src, dst) in enumerate(
        ((wk_hbm, wk_in), (wv_hbm, wv_in), (wq_hbm, wq_in), (woA_hbm, woA_in), (wqkv_hbm, wqkv_in),
         (woB_hbm, woB_in)))]
    for c in (w_cp[0], w_cp[1], x_cp[0], w_cp[2], *x_cp[1:], *w_cp[3:]):
        c.start()

    def out_copy(t):
        return pltpu.make_async_copy(out_st.at[:, _ds(t * T, T)], out_hbm.at[:, _ds(t * T, T)], out_sem.at[0])

    pacer = {"side": [], "done": 0, "time": 0.0, "total": 1.0, "gate": 0, "v": None, "slot": None}

    def tick(y, cycles, weight):
        n = max(1, cycles // 8)
        for a in range(n):
            pacer["v"] = (y, a * y.shape[0] // n // 8 * 8)
            side = pacer["side"]
            if side and pacer["gate"] < side[0][0]:
                pacer["total"] -= weight * cycles / n
                continue
            pacer["time"] += weight * cycles / n
            want = min(len(side), int(len(side) * pacer["time"] / pacer["total"]))
            while pacer["done"] < want and pacer["gate"] >= side[pacer["done"]][0]:
                side[pacer["done"]][1]()
                pacer["done"] += 1

    def pace(buf):
        if pacer["v"] is not None:
            y, r = pacer["v"]
            buf[0:8, pacer["slot"]] = y[r:r + 8, 0:T]

    def drain():
        while pacer["done"] < len(pacer["side"]):
            pacer["side"][pacer["done"]][1]()
            pacer["done"] += 1

    def run(items, side=(), tail=0):
        pacer.update(side=list(side), done=0, time=0.0, total=max(1.0, sum(c for c, _ in items) - tail),
                     gate=0, v=None)
        for _, fn in items:
            fn()
        drain()
        pacer.update(side=[], done=0)

    def fence():
        pl.semaphore_signal(bar_sem, 1)
        pl.semaphore_wait(bar_sem, 1)

    def wdot(w_ref, r0, n, x_ref):
        y = _dot(_unpack(w_ref[pl.ds(r0 // 2, n // 2), :]), _unpack(x_ref[...]))
        tick(y, n, 0.0)
        return y

    def ln_stats(st, x, first):
        if first:
            st["c"] = jnp.broadcast_to(x[0:1], (8, T))
        d = [x[i:i + 8] - st["c"] for i in range(0, x.shape[0], 8)]
        s1, s2 = _tree(jnp.add, d), _tree(jnp.add, [v * v for v in d])
        st["s1"] = s1 if first else st["s1"] + s1
        st["s2"] = s2 if first else st["s2"] + s2

    def ln_items(t, xn, st, zero, src):
        def norm():
            e1 = jnp.sum(st["s1"], axis=0, keepdims=True) * (1.0 / D)
            e2 = jnp.sum(st["s2"], axis=0, keepdims=True) * (1.0 / D)
            r = lax.rsqrt(jnp.maximum(e2 - e1 * e1, 0.0) + 1e-5)
            xn[...] = _pack((src[:, _ds(t * T + zero, T)].astype(F32) - (st["c"][0:1] + e1)) * r)
        return [(0, norm)]

    def input_norm_items(t, xn, zero):
        st = {}

        def stats():
            for g in range(NG):
                ln_stats(st, x_in[pl.ds(g * GR, GR), _ds(t * T, T)].astype(F32), g == 0)
        return [(0, stats)] + ln_items(t, xn, st, zero, x_in)

    def proj_a_items(t, kA, vA, xn):
        def kv():
            y = wdot(wA, D, 64, xn)
            kT = jnp.concatenate([_halves(y[0:DH]), jnp.zeros((96, T), F32)], axis=0)
            kA[_ds(t * (T // 2), T // 2, T // 2), :] = _pack(kT.T)[:, 0:32]
            vA[:, _ds(t * T, T)] = _pack(jnp.concatenate([y[DH:2 * DH], jnp.ones((4, T), F32)], axis=0))

        def q(g):
            def f():
                y = wdot(wA, g * GR, GR, xn) * QSCALE
                qA[:, _ds(t * (H * T) + g * GW, GW)] = _pack(
                    jnp.concatenate([_halves(y[j * DH:(j + 1) * DH]) for j in range(HG)], axis=1))
            return f
        return [(0, kv)] + [(0, q(g)) for g in range(NG)]

    def key_factor_items(kA):
        def one(kb, d):
            def f():
                k = _unpack(kA[pl.ds(kb * 16, 16), :]).astype(F32)
                lo = jnp.broadcast_to(k[:, d:d + 1], (32, 128))
                hi = jnp.broadcast_to(k[:, d + 16:d + 17], (32, 128))
                a11, a12, a21, a22 = lo[0:16], hi[0:16], lo[16:32], hi[16:32]
                s1 = a21 + a22
                s2 = s1 - a11
                b, slot = D_SLOT[d]
                for p, v in enumerate((a11, a12, a12 - s2, a22, s1, s2, a11 - a21)):
                    ops[b][:, pl.ds(QW + ((kb * 7 + p) * 4 + slot) * T, T)] = v
            return (0, f)
        return [one(kb, d) for kb in range(NV // 32) for d in D_ORDER]

    def query_factor_items(t):
        def one(g, b):
            def f():
                q, r0 = _unpack(qA[:, _ds(t * (H * T) + g * GW, GW)]).astype(F32), b % 2 * 8
                lo, hi = q[r0:r0 + 8], q[16 + r0:24 + r0]
                b11, b12, b21, b22 = lo[:, 0:256], lo[:, 256:512], hi[:, 0:256], hi[:, 256:512]
                t1 = b12 - b11
                t2 = b22 - t1
                pace(ops[b])
                for p, v in enumerate((b11, b21, b22, b21 - t2, t1, t2, b22 - b12)):
                    ops[b][0:8, pl.ds((g * 7 + p) * 2 * T, 2 * T)] = v
            return (0, f)
        return [one(g, b) for g in range(NG) for b in range(4)]

    def proj_b_items(t):
        def k(g):
            def f():
                y = wdot(wB, D + g * GR, GR, xnA)
                cur = _pack(jnp.concatenate([y, jnp.zeros((128 - GR, T), F32)], axis=0).T)
                kB[g, _ds(t * (T // 2) + WIN // 2, T // 2, T // 2), :] = cur
                w = jnp.concatenate([kB[g, _ds(t * (T // 2) + (WIN - 96) // 2, 48, 16), :], cur], axis=0)
                b0, b1 = _lane_bit(DH, 1), _lane_bit(DH, 2)
                z = [_pick(b0, w[16:112], w[0:96]), _pick(b0, w[0:96], w[16:112])]
                rows = _ds(t * (T // 2) + 80, T // 2, 16)
                for a in range(2):
                    kY[g][a, rows, :] = _pick(b1, z[a][32:96], z[a][0:64])
                    kY[g][a + 2, rows, :] = _pick(b1, z[a][0:64], z[a][32:96])
            return f

        def q(g):
            def f():
                qB[pl.ds(g * GR // 2, GR // 2), _ds(t * T, T)] = _pack(wdot(wB, g * GR, GR, xnA) * QSCALE)
            return f

        def v(g):
            def f():
                y = wdot(wB, 2 * D + g * GR, GR, xnA)
                ones = jnp.ones((4, T), F32)
                parts = []
                for j in range(HG):
                    parts += [y[j * DH:(j + 1) * DH], ones]
                vB[pl.ds(g * 64, 64), _ds(t * T + WIN, T)] = _pack(jnp.concatenate(parts, axis=0))
            return f
        return [(0, f(g)) for f in (k, q, v) for g in range(NG)]

    def out_items(t, woT, o_ref, st, src):
        def part(g):
            def f():
                rows, cols = pl.ds(g * GR, GR), _ds(t * T, T)
                x = src[rows, cols].astype(F32) + wdot(woT, g * GR, GR, o_ref)
                if st is None:
                    out_st[rows, cols] = x.astype(BF16)
                else:
                    xres[rows, cols] = x
                    ln_stats(st, x, g == 0)
            return (0, f)
        items = [part(g) for g in range(NG)]
        if st is None:
            items.append((0, lambda: out_copy(t).start()))
        return items

    def store_o(o_ref, g, acc):
        on = acc[0:DH] * pl.reciprocal(acc[DH:DH + 1])
        o_ref[_ds(g * (GR // 2), GR // 2, 8), :] = _pack(
            jnp.concatenate([on[:, j * T:(j + 1) * T] for j in range(HG)], axis=0))

    def finish_group(o_ref, g, acc):
        store_o(o_ref, g, acc)
        den = [acc[24:32, j * T:(j + 1) * T] for j in range(HG)]
        chk[0:8] = chk[0:8] + _tree(jnp.add, [acc[i:i + 8, j * T:(j + 1) * T]
                                              for i in range(0, 32, 8) for j in range(HG)])
        chk[8:16] = jnp.minimum(chk[8:16], _tree(jnp.minimum, den))
        chk[16:24] = jnp.maximum(chk[16:24], _tree(jnp.maximum, den))

    def attn_a_items(t, kA, vA, do_qk, do_pv, nv, restage=()):
        st = {}
        steps = [(g, c) for g in range(NG) for c in range(NT)]
        bound = [nv + (S - nv) * i // NT // 16 * 16 for i in range(NT + 1)]

        def pv(n):
            def f():
                g, c = steps[n]
                p = _unpack(pA[pl.ds(c * (T // 2), T // 2), pl.ds(g * GW, GW)])
                o = _dot(_unpack(vA[:, pl.ds(c * T, T)]), p)
                st["acc"] = o if c == 0 else st["acc"] + o
                pacer["gate"] = n + 1
                tick(o, 32, 1.0)
                if c == NT - 1:
                    finish_group(oA, g, st["acc"])
            return (32, f)

        def qk(n):
            g, c = steps[n]
            lo, hi = bound[c], bound[c + 1]

            def f():
                if c == 0:
                    st["q"] = _unpack(qA[:, _ds(t * (H * T) + g * GW, GW)])
                rows = pl.ds(lo // 2, (hi - lo) // 2)
                s = _dot(_unpack(kA[rows, :]), st["q"])
                pA[rows, pl.ds(g * GW, GW)] = _pack(jnp.exp2(s))
                tick(s, hi - lo, 1.0)
            return (hi - lo, f)

        def vpu_block(g, kb):
            m = {}

            def emit(r, c, s):
                pA[pl.ds(kb * 16 + r * 8, 8), pl.ds(g * GW + c * 2 * T, 2 * T)] = _pack(
                    jnp.exp2(jnp.concatenate(s, axis=1)))

            def product(p, dst, init=None, then=None):
                def one(n, d):
                    def f():
                        b, slot = D_SLOT[d]
                        if n % 2 == 0:
                            pace(ops[b])
                        kk = ops[b][:, pl.ds(QW + ((kb * 7 + p) * 4 + slot) * T, T)]
                        term = [kk * ops[b][d % 8:d % 8 + 1, pl.ds(((g * 7 + p) * 2 + j) * T, T)] for j in range(2)]
                        base = m[dst] if n else m.get(init)
                        m[dst] = term if base is None else [x + y for x, y in zip(base, term)]
                        if n == DH // 2 - 1 and then:
                            then()
                    return f
                return [one(n, d) for n, d in enumerate(D_ORDER)]

            def mix():
                emit(1, 1, [x + y for x, y in zip(m["u3"], m["m5"])])
                m["u4"] = [x + y for x, y in zip(m["u2"], m["m5"])]
            return (product(0, "m1") + product(1, "c11", "m1", lambda: emit(0, 0, m["c11"]))
                    + product(5, "u2", "m1") + product(6, "u3", "u2") + product(4, "m5", None, mix)
                    + product(2, "c12", "u4", lambda: emit(0, 1, m["c12"]))
                    + product(3, "c21", "u3", lambda: emit(1, 0, m["c21"])))

        if not do_qk:
            return [pv(n) for n in range(len(steps))], []
        ahead = -(-nv // T) if do_pv else 0
        side = []
        for g in range(NG):
            fs = [f for kb in range(nv // 32) for f in vpu_block(g, kb)] + [f for _, f in restage[4 * g:4 * g + 4]]
            side += [(g * NT + ahead if do_pv else 0, f) for f in fs]
        items = [pv(n) for n in range(ahead)]
        for n in range(len(steps)):
            if do_pv and n + ahead < len(steps):
                items.append(pv(n + ahead))
            items.append(qk(n))
        return items, side

    def attn_b_items(t, qk_b0=0, pv_c0=0):
        def qk(g):
            def f():
                qg = qB[pl.ds(g * GR // 2, GR // 2), _ds(t * T, T)]
                r0 = qk_b0 * 16
                n = BAND // 2 - r0
                for u in range(4):
                    s = _dot(_unpack(kY[g][u, _ds(t * (T // 2) + r0, n, 16), 0:GR]), _unpack(qg & qmask[u]))
                    e = jnp.exp2(s)
                    if r0:
                        e = jnp.concatenate([jnp.zeros((2 * r0, T), F32), e], axis=0)
                    pB[pl.ds((g * 4 + u) * (BAND // 4), BAND // 4), :] = _pack(
                        jnp.concatenate([e[:BAND // 2], e[BAND // 2:]], axis=1))
                tick(s, 2 * n, 0.0)
            return (0, f)

        def unskew(g):
            def f():
                odd, high = _lane_bit(32, 1), _lane_bit(32, 2)
                zb = jnp.zeros((16, 128), I32)

                def band(u):
                    w = pB[pl.ds((g * 4 + u) * (BAND // 4), BAND // 4), :]
                    return jnp.concatenate([w[0:16, 0:T] & qmask[4, 0:16], w[16:, 0:T], w[:-16, T:],
                                            w[-16:, T:] & qmask[5, 0:16]], axis=0)
                for a in range(2):
                    mid = {b: _pick(odd, jnp.concatenate([zb, band(b ^ 1)], axis=0),
                                    jnp.concatenate([band(b), zb], axis=0)) for b in (a, a + 2)}
                    for h in (a, a + 2):
                        pY[g, h] = _pick(high, jnp.concatenate([zb, zb, mid[h ^ 2]], axis=0),
                                         jnp.concatenate([mid[h], zb, zb], axis=0))
            return (0, f)

        def pv(g):
            def f():
                outs = []
                for h in range(HG):
                    v = vB[pl.ds((g * HG + h) * 16, 16), _ds((t + pv_c0) * T, (3 - pv_c0) * T)]
                    outs.append(_dot(_unpack(v), _unpack(pY[g, h, pv_c0 * 64:3 * T // 2, :])))
                tick(outs[0], 32 * (3 - pv_c0), 0.0)
                finish_group(oB, g, jnp.concatenate(outs, axis=1))
            return (0, f)
        return [[qk(g), unskew(g)] for g in range(NG)], [[pv(g)] for g in range(NG)]

    def post_a(t, src, zero):
        st = {}
        return out_items(t, woAT, oA, st, src), ln_items(t, xnA, st, zero, xres), proj_b_items(t)

    def post_b(t, last, zero):
        if last:
            return out_items(t, woBT, oB, None, xres), [], []
        st = {}
        return (out_items(t, woBT, oB, st, xres), ln_items(t, xnB, st, zero, xres),
                proj_a_items(t, kA1, vA1, xnB))

    def window(pa, qk, pv):
        return (pa[:8] + qk[0] + pa[8:9] + qk[1] + pa[9:10] + qk[2] + pa[10:11] + qk[3]
                + pv[0] + pv[1] + pv[2] + pa[11:])

    def layer_pair(r, zero0, under_first):
        kA, vA = (kA0, vA0) if r == 0 else (kA1, vA1)
        src, last = (x_in, False) if r == 0 else (xres, True)
        done = [(0, drain)]
        pacer["slot"] = _ds(zero0 + (OPW - T), T)

        main, side = attn_a_items(0, kA, vA, True, False, NV_FIRST, query_factor_items(1))
        run(under_first(main), side, 100)
        fence()

        main, side = attn_a_items(1, kA, vA, True, True, NV)
        oa, la, pa = post_a(0, src, zero0)
        qk, pv = attn_b_items(0, 5, 2)
        rest = pa[:8] + qk[0] + qk[1] + qk[2] + qk[3] + pa[8:] + pv[0] + pv[1] + pv[2]
        hold = -(-NV // T) + 1
        run(main[:-hold] + oa + la + main[-hold:] + _zip_in(rest, done + query_factor_items(2)), side)
        fence()

        def body(j, carry):
            i, zero = j + 2, (j >> 20) * T
            pacer["slot"] = _ds(zero + (OPW - T), T)
            main, side = attn_a_items(i, kA, vA, True, True, NV)
            oa, la, pa = post_a(i - 1, src, zero)
            ob, lb, pb = post_b(i - 2, last, zero)
            qk, pv = attn_b_items(i - 1)
            sq = query_factor_items(jnp.minimum(i + 1, NT - 1))
            late = attn_b_items(i - 2)[1][3]
            run(main + done + _zip_in(late + oa + la + ob, sq) + lb + window(pa, qk, pv) + pb, side, 100)
            return carry
        lax.fori_loop(0, NT - 2, body, 0)

        pacer["slot"] = _ds(zero0 + (OPW - T), T)
        main, _ = attn_a_items(None, kA, vA, False, True, NV)
        if not last:
            fence()
            run(_zip_in(main, query_factor_items(0) + key_factor_items(kA1)))
            fence()
            main = []
        oa, la, pa = post_a(NT - 1, src, zero0)
        ob, lb, pb = post_b(NT - 2, last, zero0)
        qk, pv = attn_b_items(NT - 1)
        late = attn_b_items(NT - 2)[1][3]
        run(main + late + oa + la + ob + lb + window(pa, qk, pv) + pb)
        return (pv[3],) + post_b(NT - 1, last, zero0)

    row = lax.broadcasted_iota(I32, (GR // 2, 128), 0)
    lane = lax.broadcasted_iota(I32, (GR // 2, 128), 1)
    for u in range(4):
        qmask[u] = jnp.where(((row // (DH // 2)) ^ (lane // 32)) == u, -1, 0)
    lo_w, hi_w = 0xFFFF, -0x10000
    qmask[4] = jnp.where(2 * row > lane % 32, lo_w, 0) | jnp.where(2 * row + 1 > lane % 32, hi_w, 0)
    qmask[5] = jnp.where(2 * row <= lane % 32, lo_w, 0) | jnp.where(2 * row + 1 <= lane % 32, hi_w, 0)
    chk[0:8] = jnp.zeros((8, 128), F32)
    chk[8:24] = jnp.ones((16, 128), F32)
    for g in range(NG):
        kB[g, 0:WIN // 2, :] = jnp.zeros((WIN // 2, 128), I32)
        kY[g][:, 0:80, :] = jnp.zeros((4, 80, 128), I32)
    vB[:, 0:WIN] = jnp.zeros((H * 16, WIN), I32)

    w_cp[0].wait()
    w_cp[1].wait()
    wA[D // 2:D // 2 + 32, :] = _pack(jnp.concatenate(
        [wk_in[...].astype(F32), wv_in[...].astype(F32), jnp.zeros((8, D), F32)], axis=0))
    zero0 = jnp.max(chk[0:8]).astype(I32) * T
    pacer["slot"] = _ds(zero0 + (OPW - T), T)

    def transpose_item(src, dst, i):
        def f():
            dst[pl.ds(i * D // 2, D // 2), :] = _pack(src[:, i * D:(i + 1) * D].T)
        return (0, f)

    def first_tiles(t0, t1):
        items = []
        for t in range(t0, t1):
            cur, nxt = (xnB, xnA) if t % 2 == 0 else (xnA, xnB)
            if t + 1 < NT:
                items += input_norm_items(t + 1, nxt, zero0)
            items += proj_a_items(t, kA0, vA0, cur)
        return items

    x_cp[0].wait()
    run(input_norm_items(0, xnB, zero0))
    w_cp[2].wait()
    for n in range(0, D, T):
        m = min(T, D - n)
        wA[pl.ds(n // 2, m // 2), :] = _pack(wq_in[:, n:n + m].T)
    run(first_tiles(0, X_FIRST - 1))
    x_cp[1].wait()
    run(first_tiles(X_FIRST - 1, X_SPLIT - 1))
    x_cp[2].wait()
    fence()
    run(_zip_in(first_tiles(X_SPLIT - 1, NT), query_factor_items(0) + key_factor_items(kA0)))
    fence()
    for c in w_cp[3:]:
        c.wait()
    weights = ([transpose_item(woA_in, woAT, 0)] + [transpose_item(wqkv_in, wB, i) for i in range(3)]
               + [transpose_item(woB_in, woBT, 0)])

    late, ob, lb, pb = layer_pair(0, zero0, lambda main: _zip_in(main, weights))
    late, ob, _, _ = layer_pair(1, zero0, lambda main: late + main[0:1] + ob + lb + main[1:4] + pb + main[4:])
    run(late + ob)
    for t in range(NT):
        out_copy(t).wait()

    sub = lax.broadcasted_iota(I32, (8, 128), 0)
    ok = (jnp.abs(chk[0:8]) < float("inf")) & (((chk[8:16] >= L_MIN) & (chk[16:24] <= L_MAX)) | (sub < 4))

    @pl.when(jnp.min(jnp.where(ok, 1.0, 0.0)) < 0.5)
    def _():
        def first(t, c):
            xres[:, _ds(t * T, T)] = x_in[:, _ds(t * T, T)].astype(F32)
            run(input_norm_items(t, xnB, 0) + proj_a_items(t, kA0, vA0, xnB))
            return c
        lax.fori_loop(0, NT, first, 0)

        def a_tile(t, c):
            def group(g, c):
                q = _unpack(qA[:, _ds(t * (H * T) + g * GW, GW)])

                def scores(k, m):
                    s = _dot(_unpack(kA0[_ds(k * 64, 64, 64), :]), q)
                    sX[_ds(k * T, T), :] = s
                    return jnp.maximum(m, jnp.max(s, axis=0, keepdims=True))
                m = lax.fori_loop(0, NT, scores, jnp.full((1, GW), -jnp.inf, F32))

                def weighted(k, acc):
                    p = jnp.exp2(sX[_ds(k * T, T), :] - m).astype(BF16)
                    return acc + _dot(_unpack(vA0[:, _ds(k * T, T)]), p)
                store_o(oA, g, lax.fori_loop(0, NT, weighted, jnp.zeros((32, GW), F32)))
                return c
            lax.fori_loop(0, NG, group, 0)
            oa, la, pa = post_a(t, xres, 0)
            run(oa + la + pa)
            return c

        def b_tile(t, r):
            key = lax.broadcasted_iota(I32, (3 * T, T), 0) + (t * T - WIN)
            query = lax.broadcasted_iota(I32, (3 * T, T), 1) + t * T
            valid = (key >= 0) & (key <= query) & (query - key < WIN)

            def group(g, c):
                qg = _unpack(qB[_ds(g * (GR // 2), GR // 2, 8), _ds(t * T, T)]).astype(F32)
                k = _unpack(kB[g, _ds(t * (T // 2), 3 * T // 2, 64), 0:GR])
                head = lax.broadcasted_iota(I32, (GR, T), 0) // DH
                outs = []
                for j in range(HG):
                    s = jnp.where(valid, _dot(k, jnp.where(head == j, qg, 0.0).astype(BF16)), NEG)
                    p = jnp.exp2(s - jnp.max(s, axis=0, keepdims=True)).astype(BF16)
                    outs.append(_dot(_unpack(vB[_ds((g * HG + j) * 16, 16, 16), _ds(t * T, 3 * T)]), p))
                store_o(oB, g, jnp.concatenate(outs, axis=1))
                return c
            lax.fori_loop(0, NG, group, 0)
            st = {}
            run(out_items(t, woBT, oB, st, xres))

            @pl.when(r == 0)
            def _():
                run(ln_items(t, xnB, st, 0, xres) + proj_a_items(t, kA0, vA0, xnB))
            return r

        def pair(r, c):
            lax.fori_loop(0, NT, a_tile, 0)
            lax.fori_loop(0, NT, b_tile, r)
            return c
        lax.fori_loop(0, 2, pair, 0)

        def emit(t, c):
            out_st[:, _ds(t * T, T)] = xres[:, _ds(t * T, T)].astype(BF16)
            return c
        lax.fori_loop(0, NT, emit, 0)
        cp = pltpu.make_async_copy(out_st, out_hbm, out_sem.at[0])
        cp.start()
        cp.wait()


@jax.jit
def pallas_interleave_layers__grouped_kv_mqa__sliding_block__prompt_kernel(
        A_x, A_wq, A_wk, A_wv, A_wo, B_x, B_wqkv, B_wo):
    del B_x
    out_t = pl.pallas_call(
        _kernel,
        out_shape=jax.ShapeDtypeStruct((D, S), BF16),
        in_specs=[pl.BlockSpec(memory_space=pl.ANY)] * 7,
        out_specs=pl.BlockSpec(memory_space=pl.ANY),
        scratch_shapes=[
            pltpu.VMEM((D, S), BF16),
            pltpu.VMEM((D, D), BF16),
            pltpu.VMEM((DH, D), BF16),
            pltpu.VMEM((DH, D), BF16),
            pltpu.VMEM((D, D), BF16),
            pltpu.VMEM((D, 3 * D), BF16),
            pltpu.VMEM((D, D), BF16),
            pltpu.VMEM((D, S), BF16),
            pltpu.SemaphoreType.DMA((9,)),
            pltpu.SemaphoreType.DMA((1,)),
            pltpu.SemaphoreType.REGULAR,
            pltpu.VMEM((D, S), F32),
            pltpu.VMEM((D // 2, T), I32),
            pltpu.VMEM((D // 2, T), I32),
            pltpu.VMEM((D // 2 + 32, D), I32),
            pltpu.VMEM((D // 2, D), I32),
            pltpu.VMEM((3 * D // 2, D), I32),
            pltpu.VMEM((D // 2, D), I32),
            pltpu.VMEM((S // 2, H * T), I32),
            pltpu.VMEM((NG * BAND, 2 * T), I32),
            pltpu.VMEM((NG, HG, 3 * T // 2, 128), I32),
            pltpu.VMEM((D // 2, T), I32),
            pltpu.VMEM((D // 2, T), I32),
            pltpu.VMEM((24, 128), F32),
            pltpu.VMEM((6, GR // 2, 128), I32),
            pltpu.VMEM((16, H * S), I32),
            pltpu.VMEM((S // 2, 32), I32),
            pltpu.VMEM((16, S), I32),
            pltpu.VMEM((S // 2, 32), I32),
            pltpu.VMEM((16, S), I32),
            pltpu.VMEM((D // 2, S), I32),
            pltpu.VMEM((NG, (S + WIN) // 2, 128), I32),
            pltpu.VMEM((H * 16, S + WIN), I32),
            pltpu.VMEM((S, GW), F32),
        ] + [pltpu.VMEM((16, OPW), F32)] * 4
          + [pltpu.VMEM((4, (S + 160) // 2, 128), I32)] * NG,
        compiler_params=pltpu.CompilerParams(vmem_limit_bytes=100 * 1024 * 1024),
        name="fused_layers",
    )(jnp.swapaxes(A_x[0], 0, 1), A_wq, A_wk.T, A_wv.T, A_wo, B_wqkv, B_wo)
    return jnp.swapaxes(out_t, 0, 1)[None]
```
